```python
import jax
import jax.numpy as jnp

def _softmax(x, axis=-1):
    return jax.nn.softmax(x, axis=axis)

def _gelu(x):
    return jax.nn.gelu(x, approximate=True)

def _silu(x):
    return jax.nn.silu(x)

def _sigmoid(x):
    return jax.nn.sigmoid(x)

def _layernorm(x, axis=-1, eps=1e-05):
    m = jnp.mean(x, axis=axis, keepdims=True)
    v = jnp.var(x, axis=axis, keepdims=True)
    return (x - m) / jnp.sqrt(v + eps)

def _scatter_add(tgt, idx, src, axis=0):
    return tgt.at[idx].add(src)

def _segment_sum(src, seg, n):
    return jax.ops.segment_sum(src, seg, n)

class _Rng:

    def __init__(self, key):
        self._k = key

    def _next(self):
        self._k, sub = jax.random.split(self._k)
        return sub

    def normal(self, shape):
        return jax.random.normal(self._next(), shape, dtype=jnp.bfloat16)

    def randint(self, lo, hi, shape):
        return jax.random.randint(self._next(), shape, lo, hi, dtype=jnp.int32)

    def uniform(self, shape, lo=0.0, hi=1.0):
        return jax.random.uniform(self._next(), shape, jnp.bfloat16, lo, hi)

    def permutation(self, n):
        return jax.random.permutation(self._next(), n)
kernel_name = 'sequential_preLN__memory_aug_recurrent_mem_tr__mixer_s_mlp__prompt'

def setup_inputs():
    _rng = _Rng(jax.random.key(int.from_bytes(__import__("os").urandom(4), "little")))
    _w = lambda a: (lambda t: t.astype(jnp.bfloat16) if jnp.issubdtype(t.dtype, jnp.floating) else t)(jnp.asarray(a))

    def _A_setup():
        B, S, Dm = (1, 2048, 1024)
        H, Dh = (32, 128)
        M, seg = (8, 32)
        seg = min(seg, S)
        S = S // seg * seg
        return {'x': _w((lambda *s: _rng.normal(s) * 0.05)(B, S, Dm)), 'mem0': _w((lambda *s: _rng.normal(s) * 0.05)(B, M, Dm)), 'Wq': _w((lambda *s: _rng.normal(s) * 0.05)(Dm, H, Dh) * Dm ** (-0.5)), 'Wk': _w((lambda *s: _rng.normal(s) * 0.05)(Dm, H, Dh) * Dm ** (-0.5)), 'Wv': _w((lambda *s: _rng.normal(s) * 0.05)(Dm, H, Dh) * Dm ** (-0.5)), 'Wo': _w((lambda *s: _rng.normal(s) * 0.05)(H, Dh, Dm) * (H * Dh) ** (-0.5)), 'seg_len': seg}
    _A_in = _A_setup()

    def _B_setup():
        B, S, D, F = (1, 2048, 1024, 3584)
        return {'x': _w((lambda *s: _rng.normal(s) * 0.05)(B, S, D)), 'w1': _w((lambda *s: _rng.normal(s) * 0.05)(D, D) * D ** (-0.5)), 'w2': _w((lambda *s: _rng.normal(s) * 0.05)(D, D) * D ** (-0.5)), 'w3': _w((lambda *s: _rng.normal(s) * 0.05)(D, F) * D ** (-0.5)), 'w4': _w((lambda *s: _rng.normal(s) * 0.05)(F, D) * F ** (-0.5))}
    _B_in = _B_setup()
    return {'A_x': _A_in['x'], 'A_mem0': _A_in['mem0'], 'A_Wq': _A_in['Wq'], 'A_Wk': _A_in['Wk'], 'A_Wv': _A_in['Wv'], 'A_Wo': _A_in['Wo'], 'A_seg_len': _A_in['seg_len'], 'B_x': _B_in['x'], 'B_w1': _B_in['w1'], 'B_w2': _B_in['w2'], 'B_w3': _B_in['w3'], 'B_w4': _B_in['w4']}

def reference(A_x, A_mem0, A_Wq, A_Wk, A_Wv, A_Wo, A_seg_len, B_x, B_w1, B_w2, B_w3, B_w4):

    def _A_ref(x, mem0, Wq, Wk, Wv, Wo, seg_len):
        B, S, Dm = x.shape
        H, Dh = (Wq.shape[1], Wq.shape[2])
        M = mem0.shape[1]
        scale = Dh ** (-0.5)
        n_seg = S // seg_len
        L = M + seg_len
        idx = jnp.arange(L)
        mask = (idx[:, None] < M) | (idx[:, None] >= idx[None, :])
        mem = mem0
        outs = []
        for s in range(n_seg):
            xs = x[:, s * seg_len:(s + 1) * seg_len, :].copy()
            h = jnp.concatenate([mem, xs], axis=1)
            q = jnp.einsum('btd,dhe->bhte', h, Wq)
            k = jnp.einsum('btd,dhe->bhte', h, Wk)
            v = jnp.einsum('btd,dhe->bhte', h, Wv)
            scores = jnp.einsum('bhqe,bhke->bhqk', q, k) * scale
            scores = jnp.where(mask[None, None], scores, -1000000000.0)
            p = _softmax(scores, axis=-1)
            o = jnp.einsum('bhqk,bhke->bhqe', p, v)
            o = jnp.einsum('bhte,hed->btd', o, Wo)
            mem = o[:, :M, :].copy()
            outs.append(o[:, M:, :])
        return jnp.concatenate(outs, axis=1)

    def _B_ref(x, w1, w2, w3, w4):
        B, S, D = x.shape
        h = _gelu(_layernorm(x, axis=-1) @ w1)
        c = D // 4
        g0 = jnp.pad(h[:, :, 0 * c:1 * c], ((0, 0), (1, 0), (0, 0)))[:, :S, :]
        g1 = jnp.pad(h[:, :, 1 * c:2 * c], ((0, 0), (0, 1), (0, 0)))[:, 1:, :]
        g2 = jnp.pad(h[:, :, 2 * c:3 * c], ((0, 0), (2, 0), (0, 0)))[:, :S, :]
        g3 = jnp.pad(h[:, :, 3 * c:], ((0, 0), (0, 2), (0, 0)))[:, 2:, :]
        hs = jnp.concatenate([g0, g1, g2, g3], axis=-1) @ w2
        x1 = x + hs
        h2 = _gelu(_layernorm(x1, axis=-1) @ w3) @ w4
        return x1 + h2
    x = A_x
    h = x + _A_ref(_layernorm(x, axis=-1), A_mem0, A_Wq, A_Wk, A_Wv, A_Wo, A_seg_len)
    h2 = h + _B_ref(_layernorm(h, axis=-1), B_w1, B_w2, B_w3, B_w4)
    return h2
```

```python
import functools

import jax
import jax.numpy as jnp
from jax import lax
import jax.experimental.pallas as pl
import jax.experimental.pallas.tpu as pltpu

S = 2048
D = 1024
H = 32
DH = 128
MEM = 8
SEG = 32
F = 3584
NSEG = S // SEG
L = MEM + SEG
TOK = 24
P0 = S - TOK * NSEG
RING = 576
X0 = P0 + 128
XN = 80
C4 = D // 4
HALO = 8
RB = 256
QB = RB // 4
NJ = F // 512
EPS = 1e-5
NEG = -1000000000.0

LAG_QK, LAG_PV, LAG_WO = 2, 4, 6
SPLIT = 5
UNROLL = 3

bf16 = jnp.bfloat16
f32 = jnp.float32
u32 = jnp.uint32

SEM_X0, SEM_X, SEM_WO, SEM_W1, SEM_W2, SEM_W3, SEM_W4, SEM_OUT, SEM_W = (
    0, 1, 5, 9, 13, 14, 15, 16, 20)
NSEM = SEM_W + 12


def _mult(i, n):
    return i if isinstance(i, int) else pl.multiple_of(i, n)


def _ln(x):
    m = jnp.mean(x, axis=-1, keepdims=True)
    d = x - m
    v = jnp.mean(d * d, axis=-1, keepdims=True)
    return d * lax.rsqrt(v + EPS)


def _gelu2(x):
    k = 0.7978845608028654
    return x + x * jnp.tanh(x * (k + (k * 0.044715) * (x * x)))


def _pack(x):
    return pltpu.bitcast(x.astype(bf16), u32)


def _unpack(x):
    return pltpu.bitcast(x, bf16)


def _dot(a, b):
    return jnp.dot(a, b, preferred_element_type=f32)


LHS = ((0, 3, 1), (2, 3, 1), (0, 0, 0), (3, 3, 0), (0, 1, 1), (2, 0, -1), (1, 3, -1))
RHS = ((0, 3, 1), (0, 0, 0), (1, 3, -1), (2, 0, -1), (3, 3, 0), (0, 1, 1), (2, 3, 1))
ORDER = (0, 3, 1, 5, 2, 4, 6)


LAZY = (1, 3, 4, 2, 0, 5, 6)


def _comb(pat, block):
    i, j, sign = pat
    if sign == 0:
        return block(i)
    return block(i) + block(j) if sign > 0 else block(i) - block(j)


def _rc(i, k):
    return 2 * (i >> 1) + (k >> 1), 2 * (i & 1) + (k & 1)


def _assemble(product, emit=lambda k, v: None):
    m1 = product(0)
    m4 = product(3)
    c11 = m1 + m4
    m2 = product(1)
    c21 = m2 + m4
    c22 = m1 - m2
    c22 = c22 + product(5)
    emit(2, c21)
    m3 = product(2)
    c22 = c22 + m3
    m5 = product(4)
    emit(3, c22)
    c12 = m3 + m5
    c11 = c11 - m5
    c11 = c11 + product(6)
    emit(1, c12)
    emit(0, c11)
    return c11, c12, c21, c22


def _assemble_lazy(product, emit=lambda k, v: None):
    m2 = product(1)
    m4 = product(3)
    c21 = m2 + m4
    m5 = product(4)
    emit(2, c21)
    c11 = m4 - m5
    m3 = product(2)
    c12 = m3 + m5
    c22 = m3 - m2
    m1 = product(0)
    emit(1, c12)
    c11 = c11 + m1
    c22 = c22 + m1
    c22 = c22 + product(5)
    c11 = c11 + product(6)
    emit(3, c22)
    emit(0, c11)
    return c11, c12, c21, c22


def _operands(pats, block):
    for p in range(7):
        outer = [_comb(pats[p], lambda a: block(*_rc(a, k))) for k in range(4)]
        for q in range(7):
            yield 7 * p + q, _comb(pats[q], lambda k: outer[k])


def _two_level(product, emit, inner=_assemble_lazy):
    def outer(p):
        return jnp.concatenate(inner(lambda q: product(p, q)), axis=0)

    def done(a, v):
        n = v.shape[0] // 4
        for k in (2, 1, 3, 0) if inner is _assemble_lazy else (2, 3, 1, 0):
            emit(*_rc(a, k), v[k * n:(k + 1) * n])

    _assemble_lazy(outer, done)


def _operand(pats, block):
    @functools.cache
    def outer(p, k):
        return _comb(pats[p], lambda a: block(*_rc(a, k)))

    return lambda p, q: _comb(pats[q], lambda k: outer(p, k)).astype(bf16)


def _table(i, vals):
    if isinstance(i, int):
        return vals[i]
    r = jnp.int32(vals[-1])
    for k in range(len(vals) - 2, -1, -1):
        r = jnp.where(i == k, vals[k], r)
    return r


def _attention_and_mixer(x_hbm, mem0_ref, wq_hbm, wk_hbm, wv_hbm, wo_hbm, w1_hbm, w2_hbm,
                         w3_hbm, w4_hbm, hs_, xn, kv_rings, w3b, w4b, sems,
                         wo_b, xg, w1b, w2b, *q_rings):
    w_hbm = (wq_hbm, wk_hbm, wv_hbm)
    q_r = [q_rings[h % 8].at[h // 8] for h in range(H)]

    def h_load(rows):
        return jnp.concatenate([hs_[c & 1][c >> 1, rows, :] for c in range(4)], axis=1)

    def h_store(rows, v):
        for c in range(4):
            hs_[c & 1][c >> 1, rows, :] = v[:, c * C4:(c + 1) * C4]

    def wo_copy(i):
        rows = pl.ds(_mult(i * 512, 512), 512)
        return pltpu.make_async_copy(wo_hbm.bitcast(u32).at[rows], wo_b.at[rows],
                                     sems.at[SEM_WO + i])

    w3_copies = [
        pltpu.make_async_copy(w3_hbm.bitcast(u32).at[:, pl.ds(j * 128, 128)],
                              w3b.at[pl.ds(j * D // 2, D // 2)],
                              sems.at[SEM_W3]) for j in range(4 * NJ)] + [
        pltpu.make_async_copy(w1_hbm.bitcast(u32), w1b, sems.at[SEM_W1]),
        pltpu.make_async_copy(w2_hbm.bitcast(u32), w2b, sems.at[SEM_W2])]

    def x_copies(r0, r1, sem):
        rows = pl.ds(r0 // 2, (r1 - r0) // 2)
        return [pltpu.make_async_copy(x_hbm.bitcast(u32).at[rows, pl.ds(e * 512, 512)],
                                      w4b.at[e, rows], sems.at[sem]) for e in range(2)]

    late_copies = x_copies(X0, S, SEM_X + 1)

    def norm_x(r0, n):
        rows = pl.ds(_mult(r0 // 2, 8), n // 2)
        xv = jnp.concatenate([_unpack(w4b[e, rows, :]) for e in range(2)], axis=1).astype(f32)
        h_store(pl.ds(_mult(r0, 8), n), xv)
        return _ln(xv)

    def norm_tokens(r0, n):
        xg[pl.ds(_mult(r0, 8), n), :] = norm_x(r0, n)

    def prologue(w_s, rings, lhs0):
        stg = [w3b.at[pl.ds(m * 4 * D, 4 * D)] for m in range(3)]

        def start_chunk(g, m):
            src = w_hbm[m].bitcast(u32)
            dst = stg[m].reshape(D // 2, 8, DH)
            for par in range(2):
                pltpu.make_async_copy(
                    src.at[:, pl.ds(_mult(16 * par + 4 * g, 4), 4), :],
                    dst.at[:, pl.ds(4 * par, 4), :],
                    sems.at[SEM_W + 3 * g + m]).start()

        def wait_chunk(g, m):
            pltpu.make_async_copy(stg[m], stg[m], sems.at[SEM_W + 3 * g + m]).wait()

        x0, x1 = x_copies(0, P0, SEM_X0), x_copies(P0, X0, SEM_X)
        for c in x0:
            c.start()
        start_chunk(0, 0)
        for c in x0:
            c.wait()
        start_chunk(0, 1)

        @pl.loop(0, P0 // 4 // 32)
        def _(i):
            y = [norm_x(r * (P0 // 4) + 32 * i, 32) for r in range(4)]
            for e in range(2):
                for n, v in _operands(LHS, lambda r, c: y[r][:, c * C4 + e * 128:][:, :128]):
                    lhs0[n, pl.ds(pl.multiple_of(16 * i, 16), 16), pl.ds(e * 128, 128)] = _pack(v)

        start_chunk(0, 2)
        wait_chunk(0, 0)
        for c in x1:
            c.start()

        def stage(g, m):
            count = [0]
            for e in range(2):
                seen = []

                def block(r, c):
                    w = stg[m][pl.ds(4 * C4 * r + 2 * e + (c >> 1), C4, stride=4), :]
                    w = pltpu.bitcast(w & jnp.uint32(0xFFFF0000) if c & 1 else w << 16, f32)
                    if (r, c) not in seen:
                        seen.append((r, c))
                        w_s[m][8 * g + 4 * e + c, pl.ds(r * C4 // 2, C4 // 2), :] = _pack(w)
                    return w

                b = _operand(RHS, block)

                def product(p, q):
                    res = _dot(_unpack(lhs0[7 * p + q]), b(p, q))
                    k = count[0]
                    count[0] += 1
                    if k == 73 and m < 2:
                        wait_chunk(g, m + 1)
                        if m == 1:
                            pl.when(g < 3)(functools.partial(start_chunk, g + 1, 0))
                    return res

                def emit(r, c, v):
                    rings[m * 8 + 4 * e + c][g, pl.ds(r * (P0 // 4), P0 // 4), :] = v

                _two_level(product, emit)


        @pl.loop(0, 4)
        def _(g):
            for m in range(3):
                stage(g, m)

            @pl.when(g < 3)
            def _():
                start_chunk(g + 1, 1)
                start_chunk(g + 1, 2)
                wo_copy(g).start()
                wait_chunk(g + 1, 0)

            pl.when(g == 2)(wo_copy(3).start)

        for c in x1:
            c.wait()
        norm_tokens(P0, X0 - P0)

    def wrap(r):
        return jnp.where(r >= RING, r - RING, r)

    def mixer_norm(r0, n):
        h = h_load(pl.ds(r0, n))
        d = h - jnp.mean(h, axis=-1, keepdims=True)
        var = jnp.mean(d * d, axis=-1, keepdims=True)
        inv = lax.rsqrt(var + EPS)
        v = d * inv
        for c in range(4):
            xn[c & 1][c >> 1, pl.ds(r0, n), :] = v[:, c * C4:(c + 1) * C4]
        xg[pl.ds(r0, n), :] = v * lax.rsqrt(var * inv * inv + EPS)

    def load_tok(s):
        return xg[pl.ds(pl.multiple_of(P0 + TOK * s, 8), TOK), :]

    def step(w_s, ring, s, carry, tok):
        mem, rp, ra, rw = carry
        def head_pos(axis):
            i = lax.broadcasted_iota(jnp.int32, (2 * L, 2 * L), axis)
            second = ((i >= MEM) & (i < 2 * MEM)) | (i >= 2 * MEM + SEG)
            return second, i
        (rh, ri), (ch, ci) = head_pos(0), head_pos(1)
        same = rh == ch
        mask = same & ((ri < 2 * MEM) | (ri >= ci))
        masked = jnp.where(same, NEG, -jnp.inf)

        lhs = jnp.concatenate([mem, tok], axis=0).astype(bf16)
        rps = [pl.multiple_of(wrap(rp + 8 * i), 8) for i in range(3)]
        ra_ = pl.multiple_of(ra, SEG)
        rw_ = pl.multiple_of(rw, 8)

        mem_qkv = {}
        scores = {}
        o_mem = {}
        total = [None]
        late = []

        half = D // 2
        early = {}
        for i in range(SPLIT):
            early[i // 3, i % 3] = _dot(lhs[:, :half], _unpack(w_s[i % 3][i // 3, :half // 2]))

        def qkv(h):
            res = []
            for m in range(3):
                if (h, m) in early:
                    r = _dot(lhs[:, half:], _unpack(w_s[m][h, half // 2:])) + early[h, m]
                else:
                    r = _dot(lhs, _unpack(w_s[m][h]))
                for i in range(3):
                    ring[m][h][pl.ds(rps[i], 8), :] = r[8 + 8 * i:16 + 8 * i]
                res.append(r[:MEM])
            mem_qkv[h] = res

        def both(m, h):
            return jnp.concatenate(
                [mem_qkv[h][m], mem_qkv[h + 1][m], ring[m][h][pl.ds(ra_, SEG), :],
                 ring[m][h + 1][pl.ds(ra_, SEG), :]], axis=0).astype(bf16)

        def qk(h):
            scores[h] = lax.dot_general(both(0, h), both(1, h), (((1,), (1,)), ((), ())),
                                        preferred_element_type=f32)

        def pv(h):
            va = both(2, h)
            sc = jnp.where(mask, scores.pop(h) * (DH ** -0.5), masked)
            mx = jnp.max(sc, axis=1, keepdims=True)
            e = jnp.exp(sc - mx)
            den = jnp.sum(e, axis=1, keepdims=True)
            inv = pl.reciprocal(den, approx=True)
            inv = inv * (2.0 - den * inv)
            o = _dot(e.astype(bf16), va) * inv
            for i in range(2):
                q_r[h + i][pl.ds(ra_, SEG), :] = o[2 * MEM + i * SEG:2 * MEM + (i + 1) * SEG]
                o_mem[h + i] = o[i * MEM:(i + 1) * MEM]

        def wo(h):
            lo = jnp.concatenate([o_mem.pop(h), q_r[h][pl.ds(rw_, TOK), :]],
                                 axis=0).astype(bf16)
            rows = pl.ds(h * DH // 2, DH // 2)
            if h >= H - SPLIT:
                if not late:
                    total[:] = [total[0][:, :half], total[0][:, half:]]
                late.append((lo, rows))
                total[0] = total[0] + _dot(lo, _unpack(wo_b[rows, :half]))
                return
            r = _dot(lo, _unpack(wo_b[rows, :]))
            total[0] = r if total[0] is None else total[0] + r

        npair = H // 2
        for t in range(npair + LAG_WO):
            if 0 <= t - LAG_QK < npair:
                qk(2 * (t - LAG_QK))
            if 0 <= t - LAG_PV < npair:
                pv(2 * (t - LAG_PV))
            if t < npair:
                qkv(2 * t)
                qkv(2 * t + 1)
            if 0 <= t - LAG_WO < npair:
                wo(2 * (t - LAG_WO))
                wo(2 * (t - LAG_WO) + 1)
        for lo, rows in late:
            total[1] = total[1] + _dot(lo, _unpack(wo_b[rows, half:]))
        a = jnp.concatenate(total, axis=1)
        rows = pl.ds(pl.multiple_of(TOK * s, 8), TOK)
        h_store(rows, h_load(rows) + a[MEM:])
        return a[:MEM], wrap(rp + TOK), wrap(ra + SEG), wrap(rw + TOK)

    def block_a(lhs0, wq_s, wk_s, wv_s):
        w_s = (wq_s, wk_s, wv_s)
        rings = q_rings + kv_rings
        ring = [[rings[m * 8 + h % 8].at[h // 8] for h in range(H)] for m in range(3)]
        prologue(w_s, rings, lhs0)
        for i in range(4):
            wo_copy(i).wait()
        for c in late_copies:
            c.start()

        def steps(i, carry):
            s0 = 1 + i * UNROLL
            toks = [load_tok(s0 + k) for k in range(UNROLL)]
            behind = jnp.maximum(s0 - UNROLL, 1) * TOK
            ahead = jnp.minimum(X0 + i * XN, S - XN)
            for k in range(UNROLL):
                mixer_norm(pl.multiple_of(behind + TOK * k, 8), TOK)
                if k == UNROLL - 1:
                    norm_tokens(ahead, XN)
                carry = step(w_s, ring, s0 + k, carry, toks[k])
            return carry

        carry = (mem0_ref[...].astype(f32), jnp.int32(P0), jnp.int32(0), jnp.int32(0))
        carry = step(w_s, ring, jnp.int32(0), carry, load_tok(jnp.int32(0)))
        for c in late_copies:
            c.wait()
        for c in w3_copies:
            c.start()
        lax.fori_loop(0, (NSEG - 1) // UNROLL, steps, carry)

    pl.run_scoped(block_a, pltpu.VMEM((49, P0 // 8, C4), u32),
                  *[pltpu.VMEM((H, D // 2, DH), u32)] * 3)

    def mixer(gs):
        done = TOK * NSEG

        def wo_batch():
            n = (S - done) // 4

            def lhs(r, c):
                r0 = (done + r * n) % RING
                cut = min(n, RING - r0)
                return jnp.concatenate([jnp.concatenate(
                    [ref[c, pl.ds(r0, cut), :]] + ([ref[c, pl.ds(0, n - cut), :]] if cut < n else []),
                    axis=0) for ref in q_rings], axis=1)

            a = _operand(LHS, lhs)
            b = _operand(RHS, lambda r, c: _unpack(
                wo_b[pl.ds(r * 512, 512), pl.ds(c * C4, C4)]).astype(f32))

            def emit(r, c, v):
                hs_[c & 1][c >> 1, pl.ds(done + r * n, n), :] += v

            _two_level(lambda p, q: _dot(a(p, q), b(p, q)), emit)

        def mixer_dot(first, lhs, w, emit):
            a = _operand(LHS, lambda r, c: jnp.concatenate(
                [lhs(first(r, i), c) for i in range(S // RB)], axis=0))
            b = _operand(RHS, lambda r, c: _unpack(
                w[pl.ds(r * C4 // 2, C4 // 2), pl.ds(c * C4, C4)]).astype(f32))

            def split(r, c, v):
                for i in range(S // RB):
                    for e in range(2):
                        emit(first(r, i), 2 * c + e,
                             v[i * QB:(i + 1) * QB, e * 128:(e + 1) * 128])

            _two_level(lambda p, q: _dot(a(p, q), b(p, q)), split, _assemble)

        def mixer_in():
            def emit(r0, e, v):
                gs[e, pl.ds(HALO + r0, QB), :] = _gelu2(v)

            mixer_dot(lambda r, i: (3 - r) * S // 4 + i * QB,
                      lambda r0, c: xg[pl.ds(r0, QB), pl.ds(c * C4, C4)], w1b, emit)

        def mixer_out():
            def shifted(r0, c):
                rows = pl.ds(HALO + r0 + (-1, 1, -2, 2)[c], QB)
                return jnp.concatenate([gs[2 * c + e, rows, :] for e in range(2)], axis=1)

            def emit(r0, e, v):
                ref, at = xn[e >> 1 & 1], (e >> 2, pl.ds(r0, QB), pl.ds((e & 1) * 128, 128))
                x1[r0, e] = ref[at] + 0.5 * v
                ref[at] = x1[r0, e]

            x1 = {}
            mixer_dot(lambda r, i: i * RB + r * QB, shifted, w2b, emit)
            for i in range(S // RB):
                for u in range(0, QB, 8):
                    mixer_post(i, u, lambda r0, e: x1[r0, e][u:u + 8])

        def mixer_post(i, u, x1):
            y = {r: _ln(jnp.concatenate([x1(i * RB + r * QB, e) for e in range(8)], axis=1))
                 for r in (3, 2, 1, 0)}
            for k in range(4):
                blocks = [y[r][:, c * C4:(c + 1) * C4] for r, c in (_rc(a, k) for a in range(4))]
                for p in range(7):
                    v = _comb(LHS[p], lambda a: blocks[a])
                    for e in range(2):
                        kv_rings[2 * p + e][k, pl.ds(_mult(i * QB + u, 8), 8), :] = (
                            v[:, e * 128:(e + 1) * 128])

        for c in range(8):
            for r0 in (0, HALO + S):
                gs[c, pl.ds(r0, HALO), :] = jnp.zeros((HALO, 128), f32)
        mixer_norm(0, TOK)
        mixer_norm(done - UNROLL * TOK, UNROLL * TOK)
        wo_batch()
        for r0 in range(done, S, 64):
            mixer_norm(r0, 64)
        mixer_in()
        mixer_out()

    for c in w3_copies:
        c.wait()
    pl.run_scoped(mixer, pltpu.VMEM((8, S + 2 * HALO, 128), f32))


def _kernel(*refs):
    inputs, out_hbm, (h0, h1, n0, n1, w3b, w4b, sems, *kv_rings) = refs[:10], refs[10], refs[11:]
    hs_, xn = (h0, h1), (n0, n1)
    pl.run_scoped(
        functools.partial(_attention_and_mixer, *inputs, hs_, xn, tuple(kv_rings), w3b, w4b, sems),
        pltpu.VMEM((H * DH // 2, D), u32),
        pltpu.VMEM((S, D), f32),
        pltpu.VMEM((D // 2, D), u32),
        pltpu.VMEM((D // 2, D), u32),
        *[pltpu.VMEM((H // 8, RING, DH), f32)] * 8)

    def mlp(hid, stage, *prev):
        w4_copies = [
            pltpu.make_async_copy(inputs[9].bitcast(u32).at[:, pl.ds(e * 512, 512)], w4b.at[e],
                                  sems.at[SEM_W4]) for e in range(2)]

        def up(j):
            def raw(a, k):
                r, c = _rc(a, k)
                rows = pl.ds(_mult((4 * j + c) * (D // 2) + r * 128, 128), 128)
                return _unpack(w3b[rows, :]).astype(f32)

            def y(p, k):
                return jnp.concatenate(
                    [kv_rings[2 * p + e][k, pl.ds(0, S // 4), :] for e in range(2)], axis=1)

            parts = {}
            for p in LAZY:
                w = [_comb(RHS[p], lambda a: raw(a, k)) for k in range(4)]
                parts[p] = _assemble_lazy(lambda q: _dot(
                    _comb(LHS[q], lambda k: y(p, k)).astype(bf16),
                    _comb(RHS[q], lambda k: w[k]).astype(bf16)))
            for k in (2, 3, 1, 0):
                for r0 in range(0, S // 4, 16):
                    g = [_gelu2(v) for v in _assemble_lazy(lambda p: parts[p][k][r0:r0 + 16])]
                    for p in range(7):
                        hid[p, k, j, pl.ds(r0, 16), :] = _comb(LHS[p], lambda a: g[a])

        @pl.loop(0, (NJ - 1) // 2)
        def _(i):
            @pl.when(i == 1)
            def _():
                for c in w4_copies:
                    c.start()

            for k in range(2):
                up(2 * i + k)

        def out_copy(t, k=None):
            r0, nr, c0, nc = (0, 2 * QB, 0, 2 * C4) if k is None else (
                (k >> 1) * QB, QB, (k & 1) * C4, C4)
            return pltpu.make_async_copy(
                stage.at[t, :, pl.ds(r0, nr), pl.ds(c0, nc)],
                out_hbm.at[:, t >> 1, pl.ds(r0, nr), pl.ds(_mult((t & 1) * 2 * C4 + c0, C4), nc)],
                sems.at[SEM_OUT + t])

        for c in w4_copies:
            c.wait()
        up(NJ - 1)

        def down(n, last=False):
            p = _table(n, ORDER)
            i0, i1, sg = [_table(n, [RHS[o][e] for o in ORDER]) for e in range(3)]
            sg = jnp.asarray(sg, f32)
            t = _table(n, (0, 0, 2, 3, 3, 1, 0))
            src = _table(n, (0, 0, 1, 0, 1, 0, 0))
            dst = _table(n, (0, 1, 1, 0, 0, 0, 0))
            sign = jnp.asarray(_table(n, (0, 0, 1, 1, -1, 1, -1)), f32)

            def raw(a, k, j):
                rows = pl.ds(_mult((4 * j + 2 * (a >> 1) + (k >> 1)) * 64, 64), 64)
                return _unpack(w4b[a & 1, rows, pl.ds((k & 1) * C4, C4)]).astype(f32)

            def w(k):
                return jnp.concatenate(
                    [raw(i0, k, j) + sg * raw(i1, k, j) for j in range(NJ)], axis=0)

            def product(q):
                lhs = _comb(LHS[q], lambda k: jnp.concatenate(
                    [hid[p, k, j] for j in range(NJ)], axis=1))
                return _dot(lhs.astype(bf16), _comb(RHS[q], w).astype(bf16))

            def rows(k, i):
                return pl.ds(_mult(i * RB + (2 * (t >> 1) + (k >> 1)) * QB, QB), QB)

            def gather(ref, c, k):
                return jnp.concatenate([ref[c, rows(k, i), :] for i in range(S // RB)], axis=0)

            opens = _table(n, (1, 0, 1, 1, 0, 1, 0)) > 0

            @functools.cache
            def base(k):
                return (gather(hs_[k & 1], t & 1, k)
                        + jnp.where(opens, gather(xn[k & 1], t & 1, k), 0.0)
                        + jnp.where(n > 1, sign * prev[k][src], 0.0))

            if not last:
                for k in range(4):
                    base(k)

            def emit(k, v):
                v = 0.5 * v
                if not last:
                    prev[k][dst] = v
                v = v + base(k)
                for i in range(S // RB):
                    vi = v[i * QB:(i + 1) * QB]
                    if not last:
                        hs_[k & 1][t & 1, rows(k, i), :] = vi
                    stage[t, i, pl.ds((k >> 1) * QB, QB), pl.ds((k & 1) * C4, C4)] = (
                        vi.astype(bf16))

                if last:
                    for done in {3: (2, 1, 3), 0: (0,)}.get(k, ()):
                        out_copy(t, done).start()

            _assemble_lazy(product, emit)
            return t

        @pl.loop(0, 3)
        def _(i):
            ts = [down(2 * i + k) for k in range(2)]
            for k, t in enumerate(ts):
                n = 2 * i + k
                pl.when((n == 2) | (n > 3))(out_copy(t).start)

        down(6, last=True)
        for t in range(4):
            out_copy(t).wait()

    pl.run_scoped(
        mlp,
        pltpu.VMEM((7, 4, NJ, S // 4, 128), f32),
        pltpu.VMEM((4, S // RB, RB // 2, D // 2), bf16),
        *[pltpu.VMEM((2, S // 4, C4), f32)] * 4)


@jax.jit
def pallas_sequential_preLN__memory_aug_recurrent_mem_tr__mixer_s_mlp__prompt_kernel(
    A_x: jax.Array,
    A_mem0: jax.Array,
    A_Wq: jax.Array,
    A_Wk: jax.Array,
    A_Wv: jax.Array,
    A_Wo: jax.Array,
    A_seg_len: jax.Array,
    B_x: jax.Array,
    B_w1: jax.Array,
    B_w2: jax.Array,
    B_w3: jax.Array,
    B_w4: jax.Array,
):
    del A_seg_len, B_x
    hbm = pl.BlockSpec(memory_space=pl.ANY)
    vmem = pl.BlockSpec(memory_space=pltpu.VMEM)
    scratch = [
        pltpu.VMEM((2, S, C4), f32),
        pltpu.VMEM((2, S, C4), f32),
        pltpu.VMEM((2, S, C4), f32),
        pltpu.VMEM((2, S, C4), f32),
        pltpu.VMEM((4 * NJ * D // 2, 128), u32),
        pltpu.VMEM((2, F // 2, 512), u32),
        pltpu.SemaphoreType.DMA((NSEM,)),
    ] + [pltpu.VMEM((H // 8, RING, DH), f32)] * 16
    out = pl.pallas_call(
        _kernel,
        out_shape=jax.ShapeDtypeStruct((S // RB, 2, RB // 2, D), A_x.dtype),
        in_specs=[hbm, vmem] + [hbm] * 8,
        out_specs=hbm,
        scratch_shapes=scratch,
        compiler_params=pltpu.CompilerParams(vmem_limit_bytes=128 * 1024 * 1024),
    )(A_x.reshape(S, D), A_mem0.reshape(MEM, D),
      A_Wq.reshape(D // 2, 2 * H, DH), A_Wk.reshape(D // 2, 2 * H, DH),
      A_Wv.reshape(D // 2, 2 * H, DH),
      A_Wo.reshape(H * DH, D), B_w1, B_w2, B_w3, B_w4)
    return out.reshape(A_x.shape)
```

```python
import functools

import jax
import jax.numpy as jnp
from jax import lax
import jax.experimental.pallas as pl
import jax.experimental.pallas.tpu as pltpu

S = 2048
D = 1024
H = 32
DH = 128
MEM = 8
SEG = 32
F = 3584
NSEG = S // SEG
L = MEM + SEG
TOK = 24
P0 = S - TOK * NSEG
RING = 576
XN = 48
C4 = D // 4
HALO = 8
RB = 256
QB = RB // 4
NJ = F // 512
EPS = 1e-5
NEG = -1000000000.0

LAG_QK, LAG_PV, LAG_WO = 2, 4, 6
SPLIT = 5
UNROLL = 2

bf16 = jnp.bfloat16
f32 = jnp.float32
u32 = jnp.uint32

SEM_X0, SEM_X, SEM_WO, SEM_W1, SEM_W2, SEM_W3, SEM_W4, SEM_OUT, SEM_W = (
    0, 1, 5, 9, 13, 14, 15, 16, 20)
NSEM = SEM_W + 12


def _mult(i, n):
    return i if isinstance(i, int) else pl.multiple_of(i, n)


def _ln(x):
    m = jnp.mean(x, axis=-1, keepdims=True)
    d = x - m
    v = jnp.mean(d * d, axis=-1, keepdims=True)
    return d * lax.rsqrt(v + EPS)


def _gelu2(x):
    k = 0.7978845608028654
    return x + x * jnp.tanh(x * (k + (k * 0.044715) * (x * x)))


def _pack(x):
    return pltpu.bitcast(x.astype(bf16), u32)


def _unpack(x):
    return pltpu.bitcast(x, bf16)


def _dot(a, b):
    return jnp.dot(a, b, preferred_element_type=f32)


LHS = ((0, 3, 1), (2, 3, 1), (0, 0, 0), (3, 3, 0), (0, 1, 1), (2, 0, -1), (1, 3, -1))
RHS = ((0, 3, 1), (0, 0, 0), (1, 3, -1), (2, 0, -1), (3, 3, 0), (0, 1, 1), (2, 3, 1))
ORDER = (0, 3, 1, 5, 2, 4, 6)


LAZY = (1, 3, 4, 2, 0, 5, 6)


def _comb(pat, block):
    i, j, sign = pat
    if sign == 0:
        return block(i)
    return block(i) + block(j) if sign > 0 else block(i) - block(j)


def _rc(i, k):
    return 2 * (i >> 1) + (k >> 1), 2 * (i & 1) + (k & 1)


def _assemble(product, emit=lambda k, v: None):
    m1 = product(0)
    m4 = product(3)
    c11 = m1 + m4
    m2 = product(1)
    c21 = m2 + m4
    c22 = m1 - m2
    c22 = c22 + product(5)
    emit(2, c21)
    m3 = product(2)
    c22 = c22 + m3
    m5 = product(4)
    emit(3, c22)
    c12 = m3 + m5
    c11 = c11 - m5
    c11 = c11 + product(6)
    emit(1, c12)
    emit(0, c11)
    return c11, c12, c21, c22


def _assemble_lazy(product, emit=lambda k, v: None):
    m2 = product(1)
    m4 = product(3)
    c21 = m2 + m4
    m5 = product(4)
    emit(2, c21)
    c11 = m4 - m5
    m3 = product(2)
    c12 = m3 + m5
    c22 = m3 - m2
    m1 = product(0)
    emit(1, c12)
    c11 = c11 + m1
    c22 = c22 + m1
    c22 = c22 + product(5)
    c11 = c11 + product(6)
    emit(3, c22)
    emit(0, c11)
    return c11, c12, c21, c22


def _operands(pats, block):
    for p in range(7):
        outer = [_comb(pats[p], lambda a: block(*_rc(a, k))) for k in range(4)]
        for q in range(7):
            yield 7 * p + q, _comb(pats[q], lambda k: outer[k])


def _two_level(product, emit, inner=_assemble_lazy):
    def outer(p):
        return jnp.concatenate(inner(lambda q: product(p, q)), axis=0)

    def done(a, v):
        n = v.shape[0] // 4
        for k in (2, 1, 3, 0) if inner is _assemble_lazy else (2, 3, 1, 0):
            emit(*_rc(a, k), v[k * n:(k + 1) * n])

    _assemble_lazy(outer, done)


def _operand(pats, block):
    @functools.cache
    def outer(p, k):
        return _comb(pats[p], lambda a: block(*_rc(a, k)))

    return lambda p, q: _comb(pats[q], lambda k: outer(p, k)).astype(bf16)


def _table(i, vals):
    if isinstance(i, int):
        return vals[i]
    r = jnp.int32(vals[-1])
    for k in range(len(vals) - 2, -1, -1):
        r = jnp.where(i == k, vals[k], r)
    return r


def _attention_and_mixer(x_hbm, mem0_ref, wq_hbm, wk_hbm, wv_hbm, wo_hbm, w1_hbm, w2_hbm,
                         w3_hbm, w4_hbm, hs_, xn, kv_rings, w3b, w4b, sems,
                         wo_b, xg, w1b, w2b, *q_rings):
    w_hbm = (wq_hbm, wk_hbm, wv_hbm)
    q_r = [q_rings[h % 8].at[h // 8] for h in range(H)]

    def h_load(rows):
        return jnp.concatenate([hs_[c & 1][c >> 1, rows, :] for c in range(4)], axis=1)

    def h_store(rows, v):
        for c in range(4):
            hs_[c & 1][c >> 1, rows, :] = v[:, c * C4:(c + 1) * C4]

    def wo_copy(i):
        rows = pl.ds(_mult(i * 512, 512), 512)
        return pltpu.make_async_copy(wo_hbm.bitcast(u32).at[rows], wo_b.at[rows],
                                     sems.at[SEM_WO + i])

    mlp_copies = [
        pltpu.make_async_copy(w3_hbm.bitcast(u32).at[:, pl.ds(j * 128, 128)],
                              w3b.at[pl.ds(j * D // 2, D // 2)],
                              sems.at[SEM_W3]) for j in range(4 * NJ)] + [
        pltpu.make_async_copy(w1_hbm.bitcast(u32), w1b, sems.at[SEM_W1]),
        pltpu.make_async_copy(w2_hbm.bitcast(u32), w2b, sems.at[SEM_W2])]

    def x_copies(r0, r1, sem):
        rows = pl.ds(r0 // 2, (r1 - r0) // 2)
        return [pltpu.make_async_copy(x_hbm.bitcast(u32).at[rows, pl.ds(e * 512, 512)],
                                      w4b.at[e, rows], sems.at[sem]) for e in range(2)]

    def norm_x(r0, n):
        rows = pl.ds(_mult(r0 // 2, 8), n // 2)
        xv = jnp.concatenate([_unpack(w4b[e, rows, :]) for e in range(2)], axis=1).astype(f32)
        h_store(pl.ds(_mult(r0, 8), n), xv)
        return _ln(xv)

    def norm_tokens(r0, n):
        xg[pl.ds(_mult(r0, 8), n), :] = norm_x(r0, n)

    def prologue(w_s, rings, lhs0):
        stg = [w3b.at[pl.ds(m * 4 * D, 4 * D)] for m in range(3)]

        def start_chunk(g, m):
            src = w_hbm[m].bitcast(u32)
            dst = stg[m].reshape(D // 2, 8, DH)
            for par in range(2):
                pltpu.make_async_copy(
                    src.at[:, pl.ds(_mult(16 * par + 4 * g, 4), 4), :],
                    dst.at[:, pl.ds(4 * par, 4), :],
                    sems.at[SEM_W + 3 * g + m]).start()

        def wait_chunk(g, m):
            pltpu.make_async_copy(stg[m], stg[m], sems.at[SEM_W + 3 * g + m]).wait()

        x0, x1 = x_copies(0, P0, SEM_X0), x_copies(P0, P0 + 2 * XN, SEM_X)
        for c in x0:
            c.start()
        start_chunk(0, 0)
        for c in x0:
            c.wait()
        start_chunk(0, 1)

        @pl.loop(0, P0 // 4 // 32)
        def _(i):
            y = [norm_x(r * (P0 // 4) + 32 * i, 32) for r in range(4)]
            for e in range(2):
                for n, v in _operands(LHS, lambda r, c: y[r][:, c * C4 + e * 128:][:, :128]):
                    lhs0[n, pl.ds(pl.multiple_of(16 * i, 16), 16), pl.ds(e * 128, 128)] = _pack(v)

        start_chunk(0, 2)
        wait_chunk(0, 0)

        def stage(g, m):
            count = [0]
            for e in range(2):
                seen = []

                def block(r, c):
                    w = stg[m][pl.ds(4 * C4 * r + 2 * e + (c >> 1), C4, stride=4), :]
                    w = pltpu.bitcast(w & jnp.uint32(0xFFFF0000) if c & 1 else w << 16, f32)
                    if (r, c) not in seen:
                        seen.append((r, c))
                        w_s[m][8 * g + 4 * e + c, pl.ds(r * C4 // 2, C4 // 2), :] = _pack(w)
                    return w

                b = _operand(RHS, block)

                def product(p, q):
                    res = _dot(_unpack(lhs0[7 * p + q]), b(p, q))
                    k = count[0]
                    count[0] += 1
                    if k == 73 and m < 2:
                        wait_chunk(g, m + 1)
                        if m == 1:
                            pl.when(g < 3)(functools.partial(start_chunk, g + 1, 0))
                    return res

                def emit(r, c, v):
                    rings[m * 8 + 4 * e + c][g, pl.ds(r * (P0 // 4), P0 // 4), :] = v

                _two_level(product, emit)


        @pl.loop(0, 4)
        def _(g):
            for m in range(3):
                stage(g, m)

            @pl.when(g < 3)
            def _():
                start_chunk(g + 1, 1)
                start_chunk(g + 1, 2)
                wo_copy(g).start()
                wait_chunk(g + 1, 0)

            @pl.when(g == 2)
            def _():
                wo_copy(3).start()
                for c in x1:
                    c.start()

        for c in x1:
            c.wait()
        norm_tokens(P0, XN)

    def wrap(r):
        return jnp.where(r >= RING, r - RING, r)

    def mixer_norm(r0, n):
        h = h_load(pl.ds(r0, n))
        d = h - jnp.mean(h, axis=-1, keepdims=True)
        var = jnp.mean(d * d, axis=-1, keepdims=True)
        inv = lax.rsqrt(var + EPS)
        v = d * inv
        for c in range(4):
            xn[c & 1][c >> 1, pl.ds(r0, n), :] = v[:, c * C4:(c + 1) * C4]
        xg[pl.ds(r0, n), :] = v * lax.rsqrt(var * inv * inv + EPS)

    def load_tok(s):
        return xg[pl.ds(pl.multiple_of(P0 + TOK * s, 8), TOK), :]

    def step(w_s, ring, s, carry, tok):
        mem, rp, ra, rw = carry
        def head_pos(axis):
            i = lax.broadcasted_iota(jnp.int32, (2 * L, 2 * L), axis)
            second = ((i >= MEM) & (i < 2 * MEM)) | (i >= 2 * MEM + SEG)
            return second, i
        (rh, ri), (ch, ci) = head_pos(0), head_pos(1)
        same = rh == ch
        mask = same & ((ri < 2 * MEM) | (ri >= ci))
        masked = jnp.where(same, NEG, -jnp.inf)

        lhs = jnp.concatenate([mem, tok], axis=0).astype(bf16)
        rps = [pl.multiple_of(wrap(rp + 8 * i), 8) for i in range(3)]
        ra_ = pl.multiple_of(ra, SEG)
        rw_ = pl.multiple_of(rw, 8)

        mem_qkv = {}
        scores = {}
        o_mem = {}
        total = [None]
        late = []

        half = D // 2
        early = {}
        for i in range(SPLIT):
            early[i // 3, i % 3] = _dot(lhs[:, :half], _unpack(w_s[i % 3][i // 3, :half // 2]))

        def qkv(h):
            res = []
            for m in range(3):
                if (h, m) in early:
                    r = _dot(lhs[:, half:], _unpack(w_s[m][h, half // 2:])) + early[h, m]
                else:
                    r = _dot(lhs, _unpack(w_s[m][h]))
                for i in range(3):
                    ring[m][h][pl.ds(rps[i], 8), :] = r[8 + 8 * i:16 + 8 * i]
                res.append(r[:MEM])
            mem_qkv[h] = res

        def both(m, h):
            return jnp.concatenate(
                [mem_qkv[h][m], mem_qkv[h + 1][m], ring[m][h][pl.ds(ra_, SEG), :],
                 ring[m][h + 1][pl.ds(ra_, SEG), :]], axis=0).astype(bf16)

        def qk(h):
            scores[h] = lax.dot_general(both(0, h), both(1, h), (((1,), (1,)), ((), ())),
                                        preferred_element_type=f32)

        def pv(h):
            va = both(2, h)
            sc = jnp.where(mask, scores.pop(h) * (DH ** -0.5), masked)
            mx = jnp.max(sc, axis=1, keepdims=True)
            e = jnp.exp(sc - mx)
            den = jnp.sum(e, axis=1, keepdims=True)
            inv = pl.reciprocal(den, approx=True)
            inv = inv * (2.0 - den * inv)
            o = _dot(e.astype(bf16), va) * inv
            for i in range(2):
                q_r[h + i][pl.ds(ra_, SEG), :] = o[2 * MEM + i * SEG:2 * MEM + (i + 1) * SEG]
                o_mem[h + i] = o[i * MEM:(i + 1) * MEM]

        def wo(h):
            lo = jnp.concatenate([o_mem.pop(h), q_r[h][pl.ds(rw_, TOK), :]],
                                 axis=0).astype(bf16)
            rows = pl.ds(h * DH // 2, DH // 2)
            if h >= H - SPLIT:
                if not late:
                    total[:] = [total[0][:, :half], total[0][:, half:]]
                late.append((lo, rows))
                total[0] = total[0] + _dot(lo, _unpack(wo_b[rows, :half]))
                return
            r = _dot(lo, _unpack(wo_b[rows, :]))
            total[0] = r if total[0] is None else total[0] + r

        npair = H // 2
        for t in range(npair + LAG_WO):
            if 0 <= t - LAG_QK < npair:
                qk(2 * (t - LAG_QK))
            if 0 <= t - LAG_PV < npair:
                pv(2 * (t - LAG_PV))
            if t < npair:
                qkv(2 * t)
                qkv(2 * t + 1)
            if 0 <= t - LAG_WO < npair:
                wo(2 * (t - LAG_WO))
                wo(2 * (t - LAG_WO) + 1)
        for lo, rows in late:
            total[1] = total[1] + _dot(lo, _unpack(wo_b[rows, half:]))
        a = jnp.concatenate(total, axis=1)
        rows = pl.ds(pl.multiple_of(TOK * s, 8), TOK)
        h_store(rows, h_load(rows) + a[MEM:])
        return a[:MEM], wrap(rp + TOK), wrap(ra + SEG), wrap(rw + TOK)

    def block_a(lhs0, wq_s, wk_s, wv_s):
        w_s = (wq_s, wk_s, wv_s)
        rings = q_rings + kv_rings
        ring = [[rings[m * 8 + h % 8].at[h // 8] for h in range(H)] for m in range(3)]
        prologue(w_s, rings, lhs0)
        for i in range(4):
            wo_copy(i).wait()
        x_rest = x_copies(P0 + 2 * XN, S, SEM_X + 1)
        for c in x_rest:
            c.start()

        def steps(i, carry):
            @pl.when(i == 1)
            def _():
                for c in x_rest:
                    c.wait()
                for c in mlp_copies:
                    c.start()

            s0 = i * UNROLL
            toks = [load_tok(s0 + k) for k in range(UNROLL)]
            behind = jnp.maximum(s0 - UNROLL, 0) * TOK
            ahead = jnp.minimum(P0 + (i + 1) * XN, S - XN)
            for k in range(UNROLL):
                mixer_norm(pl.multiple_of(behind + TOK * k, 8), TOK)
            for k in range(UNROLL):
                if k == UNROLL - 1:
                    norm_tokens(ahead, XN)
                carry = step(w_s, ring, s0 + k, carry, toks[k])
            return carry

        carry = (mem0_ref[...].astype(f32), jnp.int32(P0), jnp.int32(0), jnp.int32(0))
        lax.fori_loop(0, NSEG // UNROLL, steps, carry)
        for c in mlp_copies:
            c.wait()

    pl.run_scoped(block_a, pltpu.VMEM((49, P0 // 8, C4), u32),
                  *[pltpu.VMEM((H, D // 2, DH), u32)] * 3)

    def mixer(gs):
        done = TOK * NSEG

        def wo_batch():
            n = (S - done) // 4

            def lhs(r, c):
                r0 = (done + r * n) % RING
                cut = min(n, RING - r0)
                return jnp.concatenate([jnp.concatenate(
                    [ref[c, pl.ds(r0, cut), :]] + ([ref[c, pl.ds(0, n - cut), :]] if cut < n else []),
                    axis=0) for ref in q_rings], axis=1)

            a = _operand(LHS, lhs)
            b = _operand(RHS, lambda r, c: _unpack(
                wo_b[pl.ds(r * 512, 512), pl.ds(c * C4, C4)]).astype(f32))

            def emit(r, c, v):
                hs_[c & 1][c >> 1, pl.ds(done + r * n, n), :] += v

            _two_level(lambda p, q: _dot(a(p, q), b(p, q)), emit)

        def mixer_dot(first, lhs, w, emit):
            a = _operand(LHS, lambda r, c: jnp.concatenate(
                [lhs(first(r, i), c) for i in range(S // RB)], axis=0))
            b = _operand(RHS, lambda r, c: _unpack(
                w[pl.ds(r * C4 // 2, C4 // 2), pl.ds(c * C4, C4)]).astype(f32))

            def split(r, c, v):
                for i in range(S // RB):
                    for e in range(2):
                        emit(first(r, i), 2 * c + e,
                             v[i * QB:(i + 1) * QB, e * 128:(e + 1) * 128])

            _two_level(lambda p, q: _dot(a(p, q), b(p, q)), split, _assemble)

        def mixer_in():
            def emit(r0, e, v):
                gs[e, pl.ds(HALO + r0, QB), :] = _gelu2(v)

            mixer_dot(lambda r, i: (3 - r) * S // 4 + i * QB,
                      lambda r0, c: xg[pl.ds(r0, QB), pl.ds(c * C4, C4)], w1b, emit)

        def mixer_out():
            def shifted(r0, c):
                rows = pl.ds(HALO + r0 + (-1, 1, -2, 2)[c], QB)
                return jnp.concatenate([gs[2 * c + e, rows, :] for e in range(2)], axis=1)

            def emit(r0, e, v):
                ref, at = xn[e >> 1 & 1], (e >> 2, pl.ds(r0, QB), pl.ds((e & 1) * 128, 128))
                x1[r0, e] = ref[at] + 0.5 * v
                ref[at] = x1[r0, e]

            x1 = {}
            mixer_dot(lambda r, i: i * RB + r * QB, shifted, w2b, emit)
            for i in range(S // RB):
                for u in range(0, QB, 8):
                    mixer_post(i, u, lambda r0, e: x1[r0, e][u:u + 8])

        def mixer_post(i, u, x1):
            y = {r: _ln(jnp.concatenate([x1(i * RB + r * QB, e) for e in range(8)], axis=1))
                 for r in (3, 2, 1, 0)}
            for k in range(4):
                blocks = [y[r][:, c * C4:(c + 1) * C4] for r, c in (_rc(a, k) for a in range(4))]
                for p in range(7):
                    v = _comb(LHS[p], lambda a: blocks[a])
                    for e in range(2):
                        kv_rings[2 * p + e][k, pl.ds(_mult(i * QB + u, 8), 8), :] = (
                            v[:, e * 128:(e + 1) * 128])

        for c in range(8):
            for r0 in (0, HALO + S):
                gs[c, pl.ds(r0, HALO), :] = jnp.zeros((HALO, 128), f32)
        mixer_norm(done - UNROLL * TOK, UNROLL * TOK)
        wo_batch()
        for r0 in range(done, S, 64):
            mixer_norm(r0, 64)
        mixer_in()
        mixer_out()

    pl.run_scoped(mixer, pltpu.VMEM((8, S + 2 * HALO, 128), f32))


def _kernel(*refs):
    inputs, out_hbm, (h0, h1, n0, n1, w3b, w4b, sems, *kv_rings) = refs[:10], refs[10], refs[11:]
    hs_, xn = (h0, h1), (n0, n1)
    pl.run_scoped(
        functools.partial(_attention_and_mixer, *inputs, hs_, xn, tuple(kv_rings), w3b, w4b, sems),
        pltpu.VMEM((H * DH // 2, D), u32),
        pltpu.VMEM((S, D), f32),
        pltpu.VMEM((D // 2, D), u32),
        pltpu.VMEM((D // 2, D), u32),
        *[pltpu.VMEM((H // 8, RING, DH), f32)] * 8)

    def mlp(hid, stage, *prev):
        w4_copies = [
            pltpu.make_async_copy(inputs[9].bitcast(u32).at[:, pl.ds(e * 512, 512)], w4b.at[e],
                                  sems.at[SEM_W4]) for e in range(2)]

        def up(j):
            def raw(a, k):
                r, c = _rc(a, k)
                rows = pl.ds(_mult((4 * j + c) * (D // 2) + r * 128, 128), 128)
                return _unpack(w3b[rows, :]).astype(f32)

            def y(p, k):
                return jnp.concatenate(
                    [kv_rings[2 * p + e][k, pl.ds(0, S // 4), :] for e in range(2)], axis=1)

            parts = {}
            for p in LAZY:
                w = [_comb(RHS[p], lambda a: raw(a, k)) for k in range(4)]
                parts[p] = _assemble_lazy(lambda q: _dot(
                    _comb(LHS[q], lambda k: y(p, k)).astype(bf16),
                    _comb(RHS[q], lambda k: w[k]).astype(bf16)))
            for k in (2, 3, 1, 0):
                for r0 in range(0, S // 4, 16):
                    g = [_gelu2(v) for v in _assemble_lazy(lambda p: parts[p][k][r0:r0 + 16])]
                    for p in range(7):
                        hid[p, k, j, pl.ds(r0, 16), :] = _comb(LHS[p], lambda a: g[a])

        @pl.loop(0, (NJ - 1) // 2)
        def _(i):
            @pl.when(i == 1)
            def _():
                for c in w4_copies:
                    c.start()

            for k in range(2):
                up(2 * i + k)

        def out_copy(t, k=None):
            r0, nr, c0, nc = (0, 2 * QB, 0, 2 * C4) if k is None else (
                (k >> 1) * QB, QB, (k & 1) * C4, C4)
            return pltpu.make_async_copy(
                stage.at[t, :, pl.ds(r0, nr), pl.ds(c0, nc)],
                out_hbm.at[:, t >> 1, pl.ds(r0, nr), pl.ds(_mult((t & 1) * 2 * C4 + c0, C4), nc)],
                sems.at[SEM_OUT + t])

        for c in w4_copies:
            c.wait()
        up(NJ - 1)

        def down(n, last=False):
            p = _table(n, ORDER)
            i0, i1, sg = [_table(n, [RHS[o][e] for o in ORDER]) for e in range(3)]
            sg = jnp.asarray(sg, f32)
            t = _table(n, (0, 0, 2, 3, 3, 1, 0))
            src = _table(n, (0, 0, 1, 0, 1, 0, 0))
            dst = _table(n, (0, 1, 1, 0, 0, 0, 0))
            sign = jnp.asarray(_table(n, (0, 0, 1, 1, -1, 1, -1)), f32)

            def raw(a, k, j):
                rows = pl.ds(_mult((4 * j + 2 * (a >> 1) + (k >> 1)) * 64, 64), 64)
                return _unpack(w4b[a & 1, rows, pl.ds((k & 1) * C4, C4)]).astype(f32)

            def w(k):
                return jnp.concatenate(
                    [raw(i0, k, j) + sg * raw(i1, k, j) for j in range(NJ)], axis=0)

            def product(q):
                lhs = _comb(LHS[q], lambda k: jnp.concatenate(
                    [hid[p, k, j] for j in range(NJ)], axis=1))
                return _dot(lhs.astype(bf16), _comb(RHS[q], w).astype(bf16))

            def rows(k, i):
                return pl.ds(_mult(i * RB + (2 * (t >> 1) + (k >> 1)) * QB, QB), QB)

            def gather(ref, c, k):
                return jnp.concatenate([ref[c, rows(k, i), :] for i in range(S // RB)], axis=0)

            opens = _table(n, (1, 0, 1, 1, 0, 1, 0)) > 0

            @functools.cache
            def base(k):
                return (gather(hs_[k & 1], t & 1, k)
                        + jnp.where(opens, gather(xn[k & 1], t & 1, k), 0.0)
                        + jnp.where(n > 1, sign * prev[k][src], 0.0))

            if not last:
                for k in range(4):
                    base(k)

            def emit(k, v):
                v = 0.5 * v
                if not last:
                    prev[k][dst] = v
                v = v + base(k)
                for i in range(S // RB):
                    vi = v[i * QB:(i + 1) * QB]
                    if not last:
                        hs_[k & 1][t & 1, rows(k, i), :] = vi
                    stage[t, i, pl.ds((k >> 1) * QB, QB), pl.ds((k & 1) * C4, C4)] = (
                        vi.astype(bf16))

                if last:
                    for done in {3: (2, 1, 3), 0: (0,)}.get(k, ()):
                        out_copy(t, done).start()

            _assemble_lazy(product, emit)
            return t

        @pl.loop(0, 6)
        def _(n):
            pl.when((n == 2) | (n > 3))(out_copy(down(n)).start)

        down(6, last=True)
        for t in range(4):
            out_copy(t).wait()

    pl.run_scoped(
        mlp,
        pltpu.VMEM((7, 4, NJ, S // 4, 128), f32),
        pltpu.VMEM((4, S // RB, RB // 2, D // 2), bf16),
        *[pltpu.VMEM((2, S // 4, C4), f32)] * 4)


@jax.jit
def pallas_sequential_preLN__memory_aug_recurrent_mem_tr__mixer_s_mlp__prompt_kernel(
    A_x: jax.Array,
    A_mem0: jax.Array,
    A_Wq: jax.Array,
    A_Wk: jax.Array,
    A_Wv: jax.Array,
    A_Wo: jax.Array,
    A_seg_len: jax.Array,
    B_x: jax.Array,
    B_w1: jax.Array,
    B_w2: jax.Array,
    B_w3: jax.Array,
    B_w4: jax.Array,
):
    del A_seg_len, B_x
    hbm = pl.BlockSpec(memory_space=pl.ANY)
    vmem = pl.BlockSpec(memory_space=pltpu.VMEM)
    scratch = [
        pltpu.VMEM((2, S, C4), f32),
        pltpu.VMEM((2, S, C4), f32),
        pltpu.VMEM((2, S, C4), f32),
        pltpu.VMEM((2, S, C4), f32),
        pltpu.VMEM((4 * NJ * D // 2, 128), u32),
        pltpu.VMEM((2, F // 2, 512), u32),
        pltpu.SemaphoreType.DMA((NSEM,)),
    ] + [pltpu.VMEM((H // 8, RING, DH), f32)] * 16
    out = pl.pallas_call(
        _kernel,
        out_shape=jax.ShapeDtypeStruct((S // RB, 2, RB // 2, D), A_x.dtype),
        in_specs=[hbm, vmem] + [hbm] * 8,
        out_specs=hbm,
        scratch_shapes=scratch,
        compiler_params=pltpu.CompilerParams(vmem_limit_bytes=128 * 1024 * 1024),
    )(A_x.reshape(S, D), A_mem0.reshape(MEM, D),
      A_Wq.reshape(D // 2, 2 * H, DH), A_Wk.reshape(D // 2, 2 * H, DH),
      A_Wv.reshape(D // 2, 2 * H, DH),
      A_Wo.reshape(H * DH, D), B_w1, B_w2, B_w3, B_w4)
    return out.reshape(A_x.shape)
```

```python
import functools

import jax
import jax.numpy as jnp
from jax import lax
import jax.experimental.pallas as pl
import jax.experimental.pallas.tpu as pltpu

S = 2048
D = 1024
H = 32
DH = 128
MEM = 8
SEG = 32
F = 3584
NSEG = S // SEG
L = MEM + SEG
TOK = 24
P0 = S - TOK * NSEG
RING = 576
XN = 48
C4 = D // 4
HALO = 8
RB = 256
QB = RB // 4
NJ = F // 512
EPS = 1e-5
NEG = -1000000000.0

LAG_QK, LAG_PV, LAG_WO = 2, 4, 6
SPLIT = 5
UNROLL = 2

bf16 = jnp.bfloat16
f32 = jnp.float32
u32 = jnp.uint32

SEM_X0, SEM_X, SEM_WO, SEM_W1, SEM_W2, SEM_W3, SEM_W4, SEM_OUT, SEM_W = (
    0, 1, 5, 9, 13, 14, 15, 16, 20)
NSEM = SEM_W + 12


def _mult(i, n):
    return i if isinstance(i, int) else pl.multiple_of(i, n)


def _ln(x):
    m = jnp.mean(x, axis=-1, keepdims=True)
    d = x - m
    v = jnp.mean(d * d, axis=-1, keepdims=True)
    return d * lax.rsqrt(v + EPS)


def _gelu2(x):
    k = 0.7978845608028654
    return x + x * jnp.tanh(x * (k + (k * 0.044715) * (x * x)))


def _pack(x):
    return pltpu.bitcast(x.astype(bf16), u32)


def _unpack(x):
    return pltpu.bitcast(x, bf16)


def _dot(a, b):
    return jnp.dot(a, b, preferred_element_type=f32)


LHS = ((0, 3, 1), (2, 3, 1), (0, 0, 0), (3, 3, 0), (0, 1, 1), (2, 0, -1), (1, 3, -1))
RHS = ((0, 3, 1), (0, 0, 0), (1, 3, -1), (2, 0, -1), (3, 3, 0), (0, 1, 1), (2, 3, 1))
ORDER = (0, 3, 1, 5, 2, 4, 6)


LAZY = (1, 3, 4, 2, 0, 5, 6)


def _comb(pat, block):
    i, j, sign = pat
    if sign == 0:
        return block(i)
    return block(i) + block(j) if sign > 0 else block(i) - block(j)


def _rc(i, k):
    return 2 * (i >> 1) + (k >> 1), 2 * (i & 1) + (k & 1)


def _assemble(product, emit=lambda k, v: None):
    m1 = product(0)
    m4 = product(3)
    c11 = m1 + m4
    m2 = product(1)
    c21 = m2 + m4
    c22 = m1 - m2
    c22 = c22 + product(5)
    emit(2, c21)
    m3 = product(2)
    c22 = c22 + m3
    m5 = product(4)
    emit(3, c22)
    c12 = m3 + m5
    c11 = c11 - m5
    c11 = c11 + product(6)
    emit(1, c12)
    emit(0, c11)
    return c11, c12, c21, c22


def _assemble_lazy(product, emit=lambda k, v: None):
    m2 = product(1)
    m4 = product(3)
    c21 = m2 + m4
    m5 = product(4)
    emit(2, c21)
    c11 = m4 - m5
    m3 = product(2)
    c12 = m3 + m5
    c22 = m3 - m2
    m1 = product(0)
    emit(1, c12)
    c11 = c11 + m1
    c22 = c22 + m1
    c22 = c22 + product(5)
    c11 = c11 + product(6)
    emit(3, c22)
    emit(0, c11)
    return c11, c12, c21, c22


def _operands(pats, block):
    for p in range(7):
        outer = [_comb(pats[p], lambda a: block(*_rc(a, k))) for k in range(4)]
        for q in range(7):
            yield 7 * p + q, _comb(pats[q], lambda k: outer[k])


def _two_level(product, emit, inner=_assemble_lazy):
    def outer(p):
        return jnp.concatenate(inner(lambda q: product(p, q)), axis=0)

    def done(a, v):
        n = v.shape[0] // 4
        for k in (2, 1, 3, 0) if inner is _assemble_lazy else (2, 3, 1, 0):
            emit(*_rc(a, k), v[k * n:(k + 1) * n])

    _assemble_lazy(outer, done)


def _operand(pats, block):
    @functools.cache
    def outer(p, k):
        return _comb(pats[p], lambda a: block(*_rc(a, k)))

    return lambda p, q: _comb(pats[q], lambda k: outer(p, k)).astype(bf16)


def _table(i, vals):
    if isinstance(i, int):
        return vals[i]
    r = jnp.int32(vals[-1])
    for k in range(len(vals) - 2, -1, -1):
        r = jnp.where(i == k, vals[k], r)
    return r


def _attention_and_mixer(x_hbm, mem0_ref, wq_hbm, wk_hbm, wv_hbm, wo_hbm, w1_hbm, w2_hbm,
                         w3_hbm, w4_hbm, hs_, xn, kv_rings, w3b, w4b, sems,
                         wo_b, xg, w1b, w2b, *q_rings):
    w_hbm = (wq_hbm, wk_hbm, wv_hbm)
    q_r = [q_rings[h % 8].at[h // 8] for h in range(H)]

    def h_load(rows):
        return jnp.concatenate([hs_[c & 1][c >> 1, rows, :] for c in range(4)], axis=1)

    def h_store(rows, v):
        for c in range(4):
            hs_[c & 1][c >> 1, rows, :] = v[:, c * C4:(c + 1) * C4]

    def wo_copy(i):
        rows = pl.ds(_mult(i * 512, 512), 512)
        return pltpu.make_async_copy(wo_hbm.bitcast(u32).at[rows], wo_b.at[rows],
                                     sems.at[SEM_WO + i])

    mlp_copies = [
        pltpu.make_async_copy(w3_hbm.bitcast(u32).at[:, pl.ds(j * 128, 128)],
                              w3b.at[pl.ds(j * D // 2, D // 2)],
                              sems.at[SEM_W3]) for j in range(4 * NJ)] + [
        pltpu.make_async_copy(w1_hbm.bitcast(u32), w1b, sems.at[SEM_W1]),
        pltpu.make_async_copy(w2_hbm.bitcast(u32), w2b, sems.at[SEM_W2])]

    def x_copies(r0, n, sem):
        rows = pl.ds(_mult(r0 // 2, 64), n // 2)
        return [pltpu.make_async_copy(x_hbm.bitcast(u32).at[rows, pl.ds(e * 512, 512)],
                                      w4b.at[e, rows], sems.at[sem]) for e in range(2)]

    def norm_x(r0, n):
        rows = pl.ds(_mult(r0 // 2, 8), n // 2)
        xv = jnp.concatenate([_unpack(w4b[e, rows, :]) for e in range(2)], axis=1).astype(f32)
        h_store(pl.ds(_mult(r0, 8), n), xv)
        return _ln(xv)

    def norm_tokens(r0, n):
        xg[pl.ds(_mult(r0, 8), n), :] = norm_x(r0, n)

    def prologue(w_s, rings, lhs0):
        stg = [w3b.at[pl.ds(m * 4 * D, 4 * D)] for m in range(3)]

        def start_chunk(g, m):
            src = w_hbm[m].bitcast(u32)
            dst = stg[m].reshape(D // 2, 8, DH)
            for par in range(2):
                pltpu.make_async_copy(
                    src.at[:, pl.ds(_mult(16 * par + 4 * g, 4), 4), :],
                    dst.at[:, pl.ds(4 * par, 4), :],
                    sems.at[SEM_W + 3 * g + m]).start()

        def wait_chunk(g, m):
            pltpu.make_async_copy(stg[m], stg[m], sems.at[SEM_W + 3 * g + m]).wait()

        def x_part(g):
            return x_copies(P0 + g * ((S - P0) // 4), (S - P0) // 4, SEM_X + g)

        x0 = x_copies(0, P0, SEM_X0)
        for c in x0:
            c.start()
        start_chunk(0, 0)
        for c in x0:
            c.wait()
        start_chunk(0, 1)

        @pl.loop(0, P0 // 4 // 32)
        def _(i):
            y = [norm_x(r * (P0 // 4) + 32 * i, 32) for r in range(4)]
            for e in range(2):
                for n, v in _operands(LHS, lambda r, c: y[r][:, c * C4 + e * 128:][:, :128]):
                    lhs0[n, pl.ds(pl.multiple_of(16 * i, 16), 16), pl.ds(e * 128, 128)] = _pack(v)

        start_chunk(0, 2)
        wait_chunk(0, 0)
        for c in x_part(3):
            c.start()

        def stage(g, m):
            count = [0]
            for e in range(2):
                seen = []

                def block(r, c):
                    w = stg[m][pl.ds(4 * C4 * r + 2 * e + (c >> 1), C4, stride=4), :]
                    w = pltpu.bitcast(w & jnp.uint32(0xFFFF0000) if c & 1 else w << 16, f32)
                    if (r, c) not in seen:
                        seen.append((r, c))
                        w_s[m][8 * g + 4 * e + c, pl.ds(r * C4 // 2, C4 // 2), :] = _pack(w)
                    return w

                b = _operand(RHS, block)

                def product(p, q):
                    res = _dot(_unpack(lhs0[7 * p + q]), b(p, q))
                    k = count[0]
                    count[0] += 1
                    if k == 73 and m < 2:
                        wait_chunk(g, m + 1)
                        if m == 1:
                            pl.when(g < 3)(functools.partial(start_chunk, g + 1, 0))
                    return res

                def emit(r, c, v):
                    rings[m * 8 + 4 * e + c][g, pl.ds(r * (P0 // 4), P0 // 4), :] = v

                _two_level(product, emit)


        @pl.loop(0, 4)
        def _(g):
            for m in range(3):
                stage(g, m)

            @pl.when(g < 3)
            def _():
                start_chunk(g + 1, 1)
                start_chunk(g + 1, 2)
                wo_copy(g).start()
                for c in x_part(g):
                    c.start()
                wait_chunk(g + 1, 0)

            pl.when(g == 2)(wo_copy(3).start)

        for g in range(4):
            for c in x_part(g):
                c.wait()
        norm_tokens(P0, XN)

    def wrap(r):
        return jnp.where(r >= RING, r - RING, r)

    def mixer_norm(r0, n):
        h = h_load(pl.ds(r0, n))
        d = h - jnp.mean(h, axis=-1, keepdims=True)
        var = jnp.mean(d * d, axis=-1, keepdims=True)
        inv = lax.rsqrt(var + EPS)
        v = d * inv
        for c in range(4):
            xn[c & 1][c >> 1, pl.ds(r0, n), :] = v[:, c * C4:(c + 1) * C4]
        xg[pl.ds(r0, n), :] = v * lax.rsqrt(var * inv * inv + EPS)

    def load_tok(s):
        return xg[pl.ds(pl.multiple_of(P0 + TOK * s, 8), TOK), :]

    def step(w_s, ring, s, carry, tok):
        mem, rp, ra, rw = carry
        def head_pos(axis):
            i = lax.broadcasted_iota(jnp.int32, (2 * L, 2 * L), axis)
            second = ((i >= MEM) & (i < 2 * MEM)) | (i >= 2 * MEM + SEG)
            return second, i
        (rh, ri), (ch, ci) = head_pos(0), head_pos(1)
        same = rh == ch
        mask = same & ((ri < 2 * MEM) | (ri >= ci))
        masked = jnp.where(same, NEG, -jnp.inf)

        lhs = jnp.concatenate([mem, tok], axis=0).astype(bf16)
        rps = [pl.multiple_of(wrap(rp + 8 * i), 8) for i in range(3)]
        ra_ = pl.multiple_of(ra, SEG)
        rw_ = pl.multiple_of(rw, 8)

        mem_qkv = {}
        scores = {}
        o_mem = {}
        total = [None]
        late = []

        half = D // 2
        early = {}
        for i in range(SPLIT):
            early[i // 3, i % 3] = _dot(lhs[:, :half], _unpack(w_s[i % 3][i // 3, :half // 2]))

        def qkv(h):
            res = []
            for m in range(3):
                if (h, m) in early:
                    r = _dot(lhs[:, half:], _unpack(w_s[m][h, half // 2:])) + early[h, m]
                else:
                    r = _dot(lhs, _unpack(w_s[m][h]))
                for i in range(3):
                    ring[m][h][pl.ds(rps[i], 8), :] = r[8 + 8 * i:16 + 8 * i]
                res.append(r[:MEM])
            mem_qkv[h] = res

        def both(m, h):
            return jnp.concatenate(
                [mem_qkv[h][m], mem_qkv[h + 1][m], ring[m][h][pl.ds(ra_, SEG), :],
                 ring[m][h + 1][pl.ds(ra_, SEG), :]], axis=0).astype(bf16)

        def qk(h):
            scores[h] = lax.dot_general(both(0, h), both(1, h), (((1,), (1,)), ((), ())),
                                        preferred_element_type=f32)

        def pv(h):
            va = both(2, h)
            sc = jnp.where(mask, scores.pop(h) * (DH ** -0.5), masked)
            mx = jnp.max(sc, axis=1, keepdims=True)
            e = jnp.exp(sc - mx)
            den = jnp.sum(e, axis=1, keepdims=True)
            inv = pl.reciprocal(den, approx=True)
            inv = inv * (2.0 - den * inv)
            o = _dot(e.astype(bf16), va) * inv
            for i in range(2):
                q_r[h + i][pl.ds(ra_, SEG), :] = o[2 * MEM + i * SEG:2 * MEM + (i + 1) * SEG]
                o_mem[h + i] = o[i * MEM:(i + 1) * MEM]

        def wo(h):
            lo = jnp.concatenate([o_mem.pop(h), q_r[h][pl.ds(rw_, TOK), :]],
                                 axis=0).astype(bf16)
            rows = pl.ds(h * DH // 2, DH // 2)
            if h >= H - SPLIT:
                if not late:
                    total[:] = [total[0][:, :half], total[0][:, half:]]
                late.append((lo, rows))
                total[0] = total[0] + _dot(lo, _unpack(wo_b[rows, :half]))
                return
            r = _dot(lo, _unpack(wo_b[rows, :]))
            total[0] = r if total[0] is None else total[0] + r

        npair = H // 2
        for t in range(npair + LAG_WO):
            if 0 <= t - LAG_QK < npair:
                qk(2 * (t - LAG_QK))
            if 0 <= t - LAG_PV < npair:
                pv(2 * (t - LAG_PV))
            if t < npair:
                qkv(2 * t)
                qkv(2 * t + 1)
            if 0 <= t - LAG_WO < npair:
                wo(2 * (t - LAG_WO))
                wo(2 * (t - LAG_WO) + 1)
        for lo, rows in late:
            total[1] = total[1] + _dot(lo, _unpack(wo_b[rows, half:]))
        a = jnp.concatenate(total, axis=1)
        rows = pl.ds(pl.multiple_of(TOK * s, 8), TOK)
        h_store(rows, h_load(rows) + a[MEM:])
        return a[:MEM], wrap(rp + TOK), wrap(ra + SEG), wrap(rw + TOK)

    def block_a(lhs0, wq_s, wk_s, wv_s):
        w_s = (wq_s, wk_s, wv_s)
        rings = q_rings + kv_rings
        ring = [[rings[m * 8 + h % 8].at[h // 8] for h in range(H)] for m in range(3)]
        prologue(w_s, rings, lhs0)
        for i in range(4):
            wo_copy(i).wait()
        for c in mlp_copies:
            c.start()

        def steps(i, carry):
            s0 = i * UNROLL
            toks = [load_tok(s0 + k) for k in range(UNROLL)]
            behind = jnp.maximum(s0 - UNROLL, 0) * TOK
            ahead = jnp.minimum(P0 + (i + 1) * XN, S - XN)
            for k in range(UNROLL):
                mixer_norm(pl.multiple_of(behind + TOK * k, 8), TOK)
            for k in range(UNROLL):
                if k == UNROLL - 1:
                    norm_tokens(ahead, XN)
                carry = step(w_s, ring, s0 + k, carry, toks[k])
            return carry

        carry = (mem0_ref[...].astype(f32), jnp.int32(P0), jnp.int32(0), jnp.int32(0))
        lax.fori_loop(0, NSEG // UNROLL, steps, carry)
        for c in mlp_copies:
            c.wait()

    pl.run_scoped(block_a, pltpu.VMEM((49, P0 // 8, C4), u32),
                  *[pltpu.VMEM((H, D // 2, DH), u32)] * 3)

    def mixer(gs):
        done = TOK * NSEG

        def wo_batch():
            n = (S - done) // 4

            def lhs(r, c):
                r0 = (done + r * n) % RING
                cut = min(n, RING - r0)
                return jnp.concatenate([jnp.concatenate(
                    [ref[c, pl.ds(r0, cut), :]] + ([ref[c, pl.ds(0, n - cut), :]] if cut < n else []),
                    axis=0) for ref in q_rings], axis=1)

            a = _operand(LHS, lhs)
            b = _operand(RHS, lambda r, c: _unpack(
                wo_b[pl.ds(r * 512, 512), pl.ds(c * C4, C4)]).astype(f32))

            def emit(r, c, v):
                hs_[c & 1][c >> 1, pl.ds(done + r * n, n), :] += v

            _two_level(lambda p, q: _dot(a(p, q), b(p, q)), emit)

        def mixer_dot(first, lhs, w, emit):
            a = _operand(LHS, lambda r, c: jnp.concatenate(
                [lhs(first(r, i), c) for i in range(S // RB)], axis=0))
            b = _operand(RHS, lambda r, c: _unpack(
                w[pl.ds(r * C4 // 2, C4 // 2), pl.ds(c * C4, C4)]).astype(f32))

            def split(r, c, v):
                for i in range(S // RB):
                    for e in range(2):
                        emit(first(r, i), 2 * c + e,
                             v[i * QB:(i + 1) * QB, e * 128:(e + 1) * 128])

            _two_level(lambda p, q: _dot(a(p, q), b(p, q)), split, _assemble)

        def mixer_in():
            def emit(r0, e, v):
                gs[e, pl.ds(HALO + r0, QB), :] = _gelu2(v)

            mixer_dot(lambda r, i: (3 - r) * S // 4 + i * QB,
                      lambda r0, c: xg[pl.ds(r0, QB), pl.ds(c * C4, C4)], w1b, emit)

        def mixer_out():
            def shifted(r0, c):
                rows = pl.ds(HALO + r0 + (-1, 1, -2, 2)[c], QB)
                return jnp.concatenate([gs[2 * c + e, rows, :] for e in range(2)], axis=1)

            def emit(r0, e, v):
                ref, at = xn[e >> 1 & 1], (e >> 2, pl.ds(r0, QB), pl.ds((e & 1) * 128, 128))
                x1[r0, e] = ref[at] + 0.5 * v
                ref[at] = x1[r0, e]

            x1 = {}
            mixer_dot(lambda r, i: i * RB + r * QB, shifted, w2b, emit)
            for i in range(S // RB):
                for u in range(0, QB, 8):
                    mixer_post(i, u, lambda r0, e: x1[r0, e][u:u + 8])

        def mixer_post(i, u, x1):
            y = {r: _ln(jnp.concatenate([x1(i * RB + r * QB, e) for e in range(8)], axis=1))
                 for r in (3, 2, 1, 0)}
            for k in range(4):
                blocks = [y[r][:, c * C4:(c + 1) * C4] for r, c in (_rc(a, k) for a in range(4))]
                for p in range(7):
                    v = _comb(LHS[p], lambda a: blocks[a])
                    for e in range(2):
                        kv_rings[2 * p + e][k, pl.ds(_mult(i * QB + u, 8), 8), :] = (
                            v[:, e * 128:(e + 1) * 128])

        for c in range(8):
            for r0 in (0, HALO + S):
                gs[c, pl.ds(r0, HALO), :] = jnp.zeros((HALO, 128), f32)
        mixer_norm(done - UNROLL * TOK, UNROLL * TOK)
        wo_batch()
        for r0 in range(done, S, 64):
            mixer_norm(r0, 64)
        mixer_in()
        mixer_out()

    pl.run_scoped(mixer, pltpu.VMEM((8, S + 2 * HALO, 128), f32))


def _kernel(*refs):
    inputs, out_hbm, (h0, h1, n0, n1, w3b, w4b, sems, *kv_rings) = refs[:10], refs[10], refs[11:]
    hs_, xn = (h0, h1), (n0, n1)
    pl.run_scoped(
        functools.partial(_attention_and_mixer, *inputs, hs_, xn, tuple(kv_rings), w3b, w4b, sems),
        pltpu.VMEM((H * DH // 2, D), u32),
        pltpu.VMEM((S, D), f32),
        pltpu.VMEM((D // 2, D), u32),
        pltpu.VMEM((D // 2, D), u32),
        *[pltpu.VMEM((H // 8, RING, DH), f32)] * 8)

    def mlp(hid, stage, *prev):
        w4_copies = [
            pltpu.make_async_copy(inputs[9].bitcast(u32).at[:, pl.ds(e * 512, 512)], w4b.at[e],
                                  sems.at[SEM_W4]) for e in range(2)]

        def up(j):
            def raw(a, k):
                r, c = _rc(a, k)
                rows = pl.ds(_mult((4 * j + c) * (D // 2) + r * 128, 128), 128)
                return _unpack(w3b[rows, :]).astype(f32)

            def y(p, k):
                return jnp.concatenate(
                    [kv_rings[2 * p + e][k, pl.ds(0, S // 4), :] for e in range(2)], axis=1)

            parts = {}
            for p in LAZY:
                w = [_comb(RHS[p], lambda a: raw(a, k)) for k in range(4)]
                parts[p] = _assemble_lazy(lambda q: _dot(
                    _comb(LHS[q], lambda k: y(p, k)).astype(bf16),
                    _comb(RHS[q], lambda k: w[k]).astype(bf16)))
            for k in (2, 3, 1, 0):
                for r0 in range(0, S // 4, 16):
                    g = [_gelu2(v) for v in _assemble_lazy(lambda p: parts[p][k][r0:r0 + 16])]
                    for p in range(7):
                        hid[p, k, j, pl.ds(r0, 16), :] = _comb(LHS[p], lambda a: g[a])

        @pl.loop(0, NJ)
        def _(j):
            @pl.when(j == 1)
            def _():
                for c in w4_copies:
                    c.start()

            up(j)

        def out_copy(t, k=None):
            r0, nr, c0, nc = (0, 2 * QB, 0, 2 * C4) if k is None else (
                (k >> 1) * QB, QB, (k & 1) * C4, C4)
            return pltpu.make_async_copy(
                stage.at[t, :, pl.ds(r0, nr), pl.ds(c0, nc)],
                out_hbm.at[:, t >> 1, pl.ds(r0, nr), pl.ds(_mult((t & 1) * 2 * C4 + c0, C4), nc)],
                sems.at[SEM_OUT + t])

        for c in w4_copies:
            c.wait()

        def down(n, last=False):
            p = _table(n, ORDER)
            i0, i1, sg = [_table(n, [RHS[o][e] for o in ORDER]) for e in range(3)]
            sg = jnp.asarray(sg, f32)
            t = _table(n, (0, 0, 2, 3, 3, 1, 0))
            src = _table(n, (0, 0, 1, 0, 1, 0, 0))
            dst = _table(n, (0, 1, 1, 0, 0, 0, 0))
            sign = jnp.asarray(_table(n, (0, 0, 1, 1, -1, 1, -1)), f32)

            def raw(a, k, j):
                rows = pl.ds(_mult((4 * j + 2 * (a >> 1) + (k >> 1)) * 64, 64), 64)
                return _unpack(w4b[a & 1, rows, pl.ds((k & 1) * C4, C4)]).astype(f32)

            def w(k):
                return jnp.concatenate(
                    [raw(i0, k, j) + sg * raw(i1, k, j) for j in range(NJ)], axis=0)

            def product(q):
                lhs = _comb(LHS[q], lambda k: jnp.concatenate(
                    [hid[p, k, j] for j in range(NJ)], axis=1))
                return _dot(lhs.astype(bf16), _comb(RHS[q], w).astype(bf16))

            def rows(k, i):
                return pl.ds(_mult(i * RB + (2 * (t >> 1) + (k >> 1)) * QB, QB), QB)

            def gather(ref, c, k):
                return jnp.concatenate([ref[c, rows(k, i), :] for i in range(S // RB)], axis=0)

            opens = _table(n, (1, 0, 1, 1, 0, 1, 0)) > 0

            @functools.cache
            def base(k):
                return (gather(hs_[k & 1], t & 1, k)
                        + jnp.where(opens, gather(xn[k & 1], t & 1, k), 0.0)
                        + jnp.where(n > 1, sign * prev[k][src], 0.0))

            if not last:
                for k in range(4):
                    base(k)

            def emit(k, v):
                v = 0.5 * v
                if not last:
                    prev[k][dst] = v
                v = v + base(k)
                for i in range(S // RB):
                    vi = v[i * QB:(i + 1) * QB]
                    if not last:
                        hs_[k & 1][t & 1, rows(k, i), :] = vi
                    stage[t, i, pl.ds((k >> 1) * QB, QB), pl.ds((k & 1) * C4, C4)] = (
                        vi.astype(bf16))

                if last:
                    for done in {1: (2, 1), 0: (3, 0)}.get(k, ()):
                        out_copy(t, done).start()

            _assemble_lazy(product, emit)
            return t

        @pl.loop(0, 6)
        def _(n):
            pl.when((n == 2) | (n > 3))(out_copy(down(n)).start)

        down(6, last=True)
        for t in range(4):
            out_copy(t).wait()

    pl.run_scoped(
        mlp,
        pltpu.VMEM((7, 4, NJ, S // 4, 128), f32),
        pltpu.VMEM((4, S // RB, RB // 2, D // 2), bf16),
        *[pltpu.VMEM((2, S // 4, C4), f32)] * 4)


@jax.jit
def pallas_sequential_preLN__memory_aug_recurrent_mem_tr__mixer_s_mlp__prompt_kernel(
    A_x: jax.Array,
    A_mem0: jax.Array,
    A_Wq: jax.Array,
    A_Wk: jax.Array,
    A_Wv: jax.Array,
    A_Wo: jax.Array,
    A_seg_len: jax.Array,
    B_x: jax.Array,
    B_w1: jax.Array,
    B_w2: jax.Array,
    B_w3: jax.Array,
    B_w4: jax.Array,
):
    del A_seg_len, B_x
    hbm = pl.BlockSpec(memory_space=pl.ANY)
    vmem = pl.BlockSpec(memory_space=pltpu.VMEM)
    scratch = [
        pltpu.VMEM((2, S, C4), f32),
        pltpu.VMEM((2, S, C4), f32),
        pltpu.VMEM((2, S, C4), f32),
        pltpu.VMEM((2, S, C4), f32),
        pltpu.VMEM((4 * NJ * D // 2, 128), u32),
        pltpu.VMEM((2, F // 2, 512), u32),
        pltpu.SemaphoreType.DMA((NSEM,)),
    ] + [pltpu.VMEM((H // 8, RING, DH), f32)] * 16
    out = pl.pallas_call(
        _kernel,
        out_shape=jax.ShapeDtypeStruct((S // RB, 2, RB // 2, D), A_x.dtype),
        in_specs=[hbm, vmem] + [hbm] * 8,
        out_specs=hbm,
        scratch_shapes=scratch,
        compiler_params=pltpu.CompilerParams(vmem_limit_bytes=128 * 1024 * 1024),
    )(A_x.reshape(S, D), A_mem0.reshape(MEM, D),
      A_Wq.reshape(D // 2, 2 * H, DH), A_Wk.reshape(D // 2, 2 * H, DH),
      A_Wv.reshape(D // 2, 2 * H, DH),
      A_Wo.reshape(H * DH, D), B_w1, B_w2, B_w3, B_w4)
    return out.reshape(A_x.shape)
```

```python
import functools

import jax
import jax.numpy as jnp
from jax import lax
import jax.experimental.pallas as pl
import jax.experimental.pallas.tpu as pltpu

S = 2048
D = 1024
H = 32
DH = 128
MEM = 8
SEG = 32
F = 3584
NSEG = S // SEG
L = MEM + SEG
TOK = 24
P0 = S - TOK * NSEG
RING = 576
XN = 48
C4 = D // 4
HALO = 8
RB = 256
QB = RB // 4
NJ = F // 512
EPS = 1e-5
NEG = -1000000000.0

LAG_QK, LAG_PV, LAG_WO = 2, 4, 6
SPLIT = 5
UNROLL = 2

bf16 = jnp.bfloat16
f32 = jnp.float32
u32 = jnp.uint32

SEM_X0, SEM_X, SEM_WO, SEM_W1, SEM_W2, SEM_W3, SEM_W4, SEM_OUT, SEM_W = (
    0, 1, 5, 9, 13, 14, 15, 16, 20)
NSEM = SEM_W + 12


def _mult(i, n):
    return i if isinstance(i, int) else pl.multiple_of(i, n)


def _ln(x):
    m = jnp.mean(x, axis=-1, keepdims=True)
    d = x - m
    v = jnp.mean(d * d, axis=-1, keepdims=True)
    return d * lax.rsqrt(v + EPS)


def _gelu2(x):
    k = 0.7978845608028654
    return x + x * jnp.tanh(x * (k + (k * 0.044715) * (x * x)))


def _pack(x):
    return pltpu.bitcast(x.astype(bf16), u32)


def _unpack(x):
    return pltpu.bitcast(x, bf16)


def _dot(a, b):
    return jnp.dot(a, b, preferred_element_type=f32)


LHS = ((0, 3, 1), (2, 3, 1), (0, 0, 0), (3, 3, 0), (0, 1, 1), (2, 0, -1), (1, 3, -1))
RHS = ((0, 3, 1), (0, 0, 0), (1, 3, -1), (2, 0, -1), (3, 3, 0), (0, 1, 1), (2, 3, 1))
ORDER = (0, 3, 1, 5, 2, 4, 6)


LAZY = (1, 3, 4, 2, 0, 5, 6)


def _comb(pat, block):
    i, j, sign = pat
    if sign == 0:
        return block(i)
    return block(i) + block(j) if sign > 0 else block(i) - block(j)


def _rc(i, k):
    return 2 * (i >> 1) + (k >> 1), 2 * (i & 1) + (k & 1)


def _assemble(product, emit=lambda k, v: None):
    m1 = product(0)
    m4 = product(3)
    c11 = m1 + m4
    m2 = product(1)
    c21 = m2 + m4
    c22 = m1 - m2
    c22 = c22 + product(5)
    emit(2, c21)
    m3 = product(2)
    c22 = c22 + m3
    m5 = product(4)
    emit(3, c22)
    c12 = m3 + m5
    c11 = c11 - m5
    c11 = c11 + product(6)
    emit(1, c12)
    emit(0, c11)
    return c11, c12, c21, c22


def _assemble_lazy(product, emit=lambda k, v: None):
    m2 = product(1)
    m4 = product(3)
    c21 = m2 + m4
    m5 = product(4)
    emit(2, c21)
    c11 = m4 - m5
    m3 = product(2)
    c12 = m3 + m5
    c22 = m3 - m2
    m1 = product(0)
    emit(1, c12)
    c11 = c11 + m1
    c22 = c22 + m1
    c22 = c22 + product(5)
    c11 = c11 + product(6)
    emit(3, c22)
    emit(0, c11)
    return c11, c12, c21, c22


def _operands(pats, block):
    for p in range(7):
        outer = [_comb(pats[p], lambda a: block(*_rc(a, k))) for k in range(4)]
        for q in range(7):
            yield 7 * p + q, _comb(pats[q], lambda k: outer[k])


def _two_level(product, emit, inner=_assemble_lazy):
    def outer(p):
        return jnp.concatenate(inner(lambda q: product(p, q)), axis=0)

    def done(a, v):
        n = v.shape[0] // 4
        for k in (2, 1, 3, 0) if inner is _assemble_lazy else (2, 3, 1, 0):
            emit(*_rc(a, k), v[k * n:(k + 1) * n])

    _assemble_lazy(outer, done)


def _operand(pats, block):
    @functools.cache
    def outer(p, k):
        return _comb(pats[p], lambda a: block(*_rc(a, k)))

    return lambda p, q: _comb(pats[q], lambda k: outer(p, k)).astype(bf16)


def _table(i, vals):
    if isinstance(i, int):
        return vals[i]
    r = jnp.int32(vals[-1])
    for k in range(len(vals) - 2, -1, -1):
        r = jnp.where(i == k, vals[k], r)
    return r


def _attention_and_mixer(x_hbm, mem0_ref, wq_hbm, wk_hbm, wv_hbm, wo_hbm, w1_hbm, w2_hbm,
                         w3_hbm, w4_hbm, hs_, xn, kv_rings, w3b, w4b, sems,
                         wo_b, xg, w1b, w2b, *q_rings):
    w_hbm = (wq_hbm, wk_hbm, wv_hbm)
    q_r = [q_rings[h % 8].at[h // 8] for h in range(H)]

    def h_load(rows):
        return jnp.concatenate([hs_[c & 1][c >> 1, rows, :] for c in range(4)], axis=1)

    def h_store(rows, v):
        for c in range(4):
            hs_[c & 1][c >> 1, rows, :] = v[:, c * C4:(c + 1) * C4]

    def wo_copy(i):
        rows = pl.ds(_mult(i * 512, 512), 512)
        return pltpu.make_async_copy(wo_hbm.bitcast(u32).at[rows], wo_b.at[rows],
                                     sems.at[SEM_WO + i])

    mlp_copies = [
        pltpu.make_async_copy(w3_hbm.bitcast(u32).at[:, pl.ds(j * 128, 128)],
                              w3b.at[pl.ds(j * D // 2, D // 2)],
                              sems.at[SEM_W3]) for j in range(4 * NJ)] + [
        pltpu.make_async_copy(w1_hbm.bitcast(u32), w1b, sems.at[SEM_W1]),
        pltpu.make_async_copy(w2_hbm.bitcast(u32), w2b, sems.at[SEM_W2])]

    def x_copies(r0, n, sem):
        rows = pl.ds(_mult(r0 // 2, 64), n // 2)
        return [pltpu.make_async_copy(x_hbm.bitcast(u32).at[rows, pl.ds(e * 512, 512)],
                                      w4b.at[e, rows], sems.at[sem]) for e in range(2)]

    def norm_x(r0, n):
        rows = pl.ds(_mult(r0 // 2, 8), n // 2)
        xv = jnp.concatenate([_unpack(w4b[e, rows, :]) for e in range(2)], axis=1).astype(f32)
        h_store(pl.ds(_mult(r0, 8), n), xv)
        return _ln(xv)

    def norm_tokens(r0, n):
        xg[pl.ds(_mult(r0, 8), n), :] = norm_x(r0, n)

    def prologue(w_s, rings, lhs0):
        stg = [w3b.at[pl.ds(m * 4 * D, 4 * D)] for m in range(3)]

        def start_chunk(g, m):
            src = w_hbm[m].bitcast(u32)
            dst = w3b.reshape(w3b.shape[0] // 8, 8, DH)
            for par in range(2):
                pltpu.make_async_copy(
                    src.at[:, pl.ds(_mult(16 * par + 4 * g, 4), 4), :],
                    dst.at[pl.ds(m * D // 2, D // 2), pl.ds(4 * par, 4), :],
                    sems.at[SEM_W + 3 * g + m]).start()

        def wait_chunk(g, m):
            pltpu.make_async_copy(stg[m], stg[m], sems.at[SEM_W + 3 * g + m]).wait()

        def x_part(g):
            return x_copies(P0 + g * ((S - P0) // 4), (S - P0) // 4, SEM_X + g)

        x0 = x_copies(0, P0, SEM_X0)
        for c in x0:
            c.start()
        start_chunk(0, 0)
        for c in x0:
            c.wait()
        start_chunk(0, 1)

        @pl.loop(0, P0 // 4 // 32)
        def _(i):
            y = [norm_x(r * (P0 // 4) + 32 * i, 32) for r in range(4)]
            for e in range(2):
                for n, v in _operands(LHS, lambda r, c: y[r][:, c * C4 + e * 128:][:, :128]):
                    lhs0[n, pl.ds(pl.multiple_of(16 * i, 16), 16), pl.ds(e * 128, 128)] = _pack(v)

        start_chunk(0, 2)
        wait_chunk(0, 0)
        for c in x_part(3):
            c.start()

        def stage(g, m):
            count = [0]
            for e in range(2):
                seen = []

                def block(r, c):
                    at = (8 * g + 4 * e + c, pl.ds(r * C4 // 2, C4 // 2), slice(None))
                    if (r, c) in seen:
                        return _unpack(w_s[m][at]).astype(f32)
                    seen.append((r, c))
                    w = w3b[pl.ds(4 * D * m + 4 * C4 * r + 2 * e + (c >> 1), C4, stride=4), :]
                    w = pltpu.bitcast(w & jnp.uint32(0xFFFF0000) if c & 1 else w << 16, f32)
                    w_s[m][at] = _pack(w)
                    return w

                b = _operand(RHS, block)

                def product(p, q):
                    res = _dot(_unpack(lhs0[7 * p + q]), b(p, q))
                    k = count[0]
                    count[0] += 1
                    if k == 73 and m < 2:
                        wait_chunk(g, m + 1)
                        if m == 1:
                            pl.when(g < 3)(functools.partial(start_chunk, g + 1, 0))
                    return res

                def emit(r, c, v):
                    rings[m * 8 + 4 * e + c][g, pl.ds(r * (P0 // 4), P0 // 4), :] = v

                _two_level(product, emit)


        @pl.loop(0, 4)
        def _(g):
            for m in range(3):
                stage(g, m)

            @pl.when(g < 3)
            def _():
                start_chunk(g + 1, 1)
                start_chunk(g + 1, 2)
                wo_copy(g).start()
                for c in x_part(g):
                    c.start()
                wait_chunk(g + 1, 0)

            pl.when(g == 2)(wo_copy(3).start)

        for g in range(4):
            for c in x_part(g):
                c.wait()
        norm_tokens(P0, XN)

    def wrap(r):
        return jnp.where(r >= RING, r - RING, r)

    def mixer_norm(r0, n):
        h = h_load(pl.ds(r0, n))
        d = h - jnp.mean(h, axis=-1, keepdims=True)
        var = jnp.mean(d * d, axis=-1, keepdims=True)
        inv = lax.rsqrt(var + EPS)
        v = d * inv
        for c in range(4):
            xn[c & 1][c >> 1, pl.ds(r0, n), :] = v[:, c * C4:(c + 1) * C4]
        xg[pl.ds(r0, n), :] = v * lax.rsqrt(var * inv * inv + EPS)

    def load_tok(s):
        return xg[pl.ds(pl.multiple_of(P0 + TOK * s, 8), TOK), :]

    def step(w_s, ring, s, carry, tok):
        mem, rp, ra, rw = carry
        def head_pos(axis):
            i = lax.broadcasted_iota(jnp.int32, (2 * L, 2 * L), axis)
            second = ((i >= MEM) & (i < 2 * MEM)) | (i >= 2 * MEM + SEG)
            return second, i
        (rh, ri), (ch, ci) = head_pos(0), head_pos(1)
        same = rh == ch
        mask = same & ((ri < 2 * MEM) | (ri >= ci))
        masked = jnp.where(same, NEG, -jnp.inf)

        lhs = jnp.concatenate([mem, tok], axis=0).astype(bf16)
        rps = [pl.multiple_of(wrap(rp + 8 * i), 8) for i in range(3)]
        ra_ = pl.multiple_of(ra, SEG)
        rw_ = pl.multiple_of(rw, 8)

        mem_qkv = {}
        scores = {}
        o_mem = {}
        total = [None]
        late = []

        half = D // 2
        early = {}
        for i in range(SPLIT):
            early[i // 3, i % 3] = _dot(lhs[:, :half], _unpack(w_s[i % 3][i // 3, :half // 2]))

        def qkv(h):
            res = []
            for m in range(3):
                if (h, m) in early:
                    r = _dot(lhs[:, half:], _unpack(w_s[m][h, half // 2:])) + early[h, m]
                else:
                    r = _dot(lhs, _unpack(w_s[m][h]))
                for i in range(3):
                    ring[m][h][pl.ds(rps[i], 8), :] = r[8 + 8 * i:16 + 8 * i]
                res.append(r[:MEM])
            mem_qkv[h] = res

        def both(m, h):
            return jnp.concatenate(
                [mem_qkv[h][m], mem_qkv[h + 1][m], ring[m][h][pl.ds(ra_, SEG), :],
                 ring[m][h + 1][pl.ds(ra_, SEG), :]], axis=0).astype(bf16)

        def qk(h):
            scores[h] = lax.dot_general(both(0, h), both(1, h), (((1,), (1,)), ((), ())),
                                        preferred_element_type=f32)

        def pv(h):
            va = both(2, h)
            sc = jnp.where(mask, scores.pop(h) * (DH ** -0.5), masked)
            mx = jnp.max(sc, axis=1, keepdims=True)
            e = jnp.exp(sc - mx)
            den = jnp.sum(e, axis=1, keepdims=True)
            inv = pl.reciprocal(den, approx=True)
            inv = inv * (2.0 - den * inv)
            o = _dot(e.astype(bf16), va) * inv
            for i in range(2):
                q_r[h + i][pl.ds(ra_, SEG), :] = o[2 * MEM + i * SEG:2 * MEM + (i + 1) * SEG]
                o_mem[h + i] = o[i * MEM:(i + 1) * MEM]

        def wo(h):
            lo = jnp.concatenate([o_mem.pop(h), q_r[h][pl.ds(rw_, TOK), :]],
                                 axis=0).astype(bf16)
            rows = pl.ds(h * DH // 2, DH // 2)
            if h >= H - SPLIT:
                if not late:
                    total[:] = [total[0][:, :half], total[0][:, half:]]
                late.append((lo, rows))
                total[0] = total[0] + _dot(lo, _unpack(wo_b[rows, :half]))
                return
            r = _dot(lo, _unpack(wo_b[rows, :]))
            total[0] = r if total[0] is None else total[0] + r

        npair = H // 2
        for t in range(npair + LAG_WO):
            if 0 <= t - LAG_QK < npair:
                qk(2 * (t - LAG_QK))
            if 0 <= t - LAG_PV < npair:
                pv(2 * (t - LAG_PV))
            if t < npair:
                qkv(2 * t)
                qkv(2 * t + 1)
            if 0 <= t - LAG_WO < npair:
                wo(2 * (t - LAG_WO))
                wo(2 * (t - LAG_WO) + 1)
        for lo, rows in late:
            total[1] = total[1] + _dot(lo, _unpack(wo_b[rows, half:]))
        a = jnp.concatenate(total, axis=1)
        rows = pl.ds(pl.multiple_of(TOK * s, 8), TOK)
        h_store(rows, h_load(rows) + a[MEM:])
        return a[:MEM], wrap(rp + TOK), wrap(ra + SEG), wrap(rw + TOK)

    def block_a(lhs0, wq_s, wk_s, wv_s):
        w_s = (wq_s, wk_s, wv_s)
        rings = q_rings + kv_rings
        ring = [[rings[m * 8 + h % 8].at[h // 8] for h in range(H)] for m in range(3)]
        prologue(w_s, rings, lhs0)
        for i in range(4):
            wo_copy(i).wait()
        for c in mlp_copies:
            c.start()

        def steps(i, carry):
            s0 = i * UNROLL
            toks = [load_tok(s0 + k) for k in range(UNROLL)]
            behind = jnp.maximum(s0 - UNROLL, 0) * TOK
            ahead = jnp.minimum(P0 + (i + 1) * XN, S - XN)
            for k in range(UNROLL):
                mixer_norm(pl.multiple_of(behind + TOK * k, 8), TOK)
            for k in range(UNROLL):
                if k == UNROLL - 1:
                    norm_tokens(ahead, XN)
                carry = step(w_s, ring, s0 + k, carry, toks[k])
            return carry

        carry = (mem0_ref[...].astype(f32), jnp.int32(P0), jnp.int32(0), jnp.int32(0))
        lax.fori_loop(0, NSEG // UNROLL, steps, carry)
        for c in mlp_copies:
            c.wait()

    pl.run_scoped(block_a, pltpu.VMEM((49, P0 // 8, C4), u32),
                  *[pltpu.VMEM((H, D // 2, DH), u32)] * 3)

    def mixer(gs):
        done = TOK * NSEG

        def wo_batch():
            n = (S - done) // 4

            def lhs(r, c):
                r0 = (done + r * n) % RING
                cut = min(n, RING - r0)
                return jnp.concatenate([jnp.concatenate(
                    [ref[c, pl.ds(r0, cut), :]] + ([ref[c, pl.ds(0, n - cut), :]] if cut < n else []),
                    axis=0) for ref in q_rings], axis=1)

            a = _operand(LHS, lhs)
            b = _operand(RHS, lambda r, c: _unpack(
                wo_b[pl.ds(r * 512, 512), pl.ds(c * C4, C4)]).astype(f32))

            def emit(r, c, v):
                hs_[c & 1][c >> 1, pl.ds(done + r * n, n), :] += v

            _two_level(lambda p, q: _dot(a(p, q), b(p, q)), emit)

        def mixer_dot(first, lhs, w, emit):
            a = _operand(LHS, lambda r, c: jnp.concatenate(
                [lhs(first(r, i), c) for i in range(S // RB)], axis=0))
            b = _operand(RHS, lambda r, c: _unpack(
                w[pl.ds(r * C4 // 2, C4 // 2), pl.ds(c * C4, C4)]).astype(f32))

            def split(r, c, v):
                for i in range(S // RB):
                    for e in range(2):
                        emit(first(r, i), 2 * c + e,
                             v[i * QB:(i + 1) * QB, e * 128:(e + 1) * 128])

            _two_level(lambda p, q: _dot(a(p, q), b(p, q)), split, _assemble)

        def mixer_in():
            def emit(r0, e, v):
                gs[e, pl.ds(HALO + r0, QB), :] = _gelu2(v)

            mixer_dot(lambda r, i: (3 - r) * S // 4 + i * QB,
                      lambda r0, c: xg[pl.ds(r0, QB), pl.ds(c * C4, C4)], w1b, emit)

        def mixer_out():
            def shifted(r0, c):
                rows = pl.ds(HALO + r0 + (-1, 1, -2, 2)[c], QB)
                return jnp.concatenate([gs[2 * c + e, rows, :] for e in range(2)], axis=1)

            def emit(r0, e, v):
                ref, at = xn[e >> 1 & 1], (e >> 2, pl.ds(r0, QB), pl.ds((e & 1) * 128, 128))
                x1[r0, e] = ref[at] + 0.5 * v
                ref[at] = x1[r0, e]

            x1 = {}
            mixer_dot(lambda r, i: i * RB + r * QB, shifted, w2b, emit)
            for i in range(S // RB):
                for u in range(0, QB, 8):
                    mixer_post(i, u, lambda r0, e: x1[r0, e][u:u + 8])

        def mixer_post(i, u, x1):
            y = {r: _ln(jnp.concatenate([x1(i * RB + r * QB, e) for e in range(8)], axis=1))
                 for r in (3, 2, 1, 0)}
            for k in range(4):
                blocks = [y[r][:, c * C4:(c + 1) * C4] for r, c in (_rc(a, k) for a in range(4))]
                for p in range(7):
                    v = _comb(LHS[p], lambda a: blocks[a])
                    for e in range(2):
                        kv_rings[2 * p + e][k, pl.ds(_mult(i * QB + u, 8), 8), :] = (
                            v[:, e * 128:(e + 1) * 128])

        for c in range(8):
            for r0 in (0, HALO + S):
                gs[c, pl.ds(r0, HALO), :] = jnp.zeros((HALO, 128), f32)
        mixer_norm(done - UNROLL * TOK, UNROLL * TOK)
        wo_batch()
        for r0 in range(done, S, 64):
            mixer_norm(r0, 64)
        mixer_in()
        mixer_out()

    pl.run_scoped(mixer, pltpu.VMEM((8, S + 2 * HALO, 128), f32))


def _kernel(*refs):
    inputs, out_hbm, (h0, h1, n0, n1, w3b, w4b, sems, *kv_rings) = refs[:10], refs[10], refs[11:]
    hs_, xn = (h0, h1), (n0, n1)
    pl.run_scoped(
        functools.partial(_attention_and_mixer, *inputs, hs_, xn, tuple(kv_rings), w3b, w4b, sems),
        pltpu.VMEM((H * DH // 2, D), u32),
        pltpu.VMEM((S, D), f32),
        pltpu.VMEM((D // 2, D), u32),
        pltpu.VMEM((D // 2, D), u32),
        *[pltpu.VMEM((H // 8, RING, DH), f32)] * 8)

    def mlp(hid, stage, *prev):
        w4_copies = [
            pltpu.make_async_copy(inputs[9].bitcast(u32).at[:, pl.ds(e * 512, 512)], w4b.at[e],
                                  sems.at[SEM_W4]) for e in range(2)]

        def up(j):
            def raw(a, k):
                r, c = _rc(a, k)
                rows = pl.ds(_mult((4 * j + c) * (D // 2) + r * 128, 128), 128)
                return _unpack(w3b[rows, :]).astype(f32)

            def y(p, k):
                return jnp.concatenate(
                    [kv_rings[2 * p + e][k, pl.ds(0, S // 4), :] for e in range(2)], axis=1)

            parts = {}
            for p in LAZY:
                w = [_comb(RHS[p], lambda a: raw(a, k)) for k in range(4)]
                parts[p] = _assemble_lazy(lambda q: _dot(
                    _comb(LHS[q], lambda k: y(p, k)).astype(bf16),
                    _comb(RHS[q], lambda k: w[k]).astype(bf16)))
            for k in (2, 3, 1, 0):
                for r0 in range(0, S // 4, 16):
                    g = [_gelu2(v) for v in _assemble_lazy(lambda p: parts[p][k][r0:r0 + 16])]
                    for p in range(7):
                        hid[p, k, j, pl.ds(r0, 16), :] = _comb(LHS[p], lambda a: g[a])

        @pl.loop(0, NJ)
        def _(j):
            @pl.when(j == 1)
            def _():
                for c in w4_copies:
                    c.start()

            up(j)

        def out_copy(t, k=None):
            r0, nr, c0, nc = (0, 2 * QB, 0, 2 * C4) if k is None else (
                (k >> 1) * QB, QB, (k & 1) * C4, C4)
            return pltpu.make_async_copy(
                stage.at[t, :, pl.ds(r0, nr), pl.ds(c0, nc)],
                out_hbm.at[:, t >> 1, pl.ds(r0, nr), pl.ds(_mult((t & 1) * 2 * C4 + c0, C4), nc)],
                sems.at[SEM_OUT + t])

        for c in w4_copies:
            c.wait()

        def down(n, last=False):
            p = _table(n, ORDER)
            i0, i1, sg = [_table(n, [RHS[o][e] for o in ORDER]) for e in range(3)]
            sg = jnp.asarray(sg, f32)
            t = _table(n, (0, 0, 2, 3, 3, 1, 0))
            src = _table(n, (0, 0, 1, 0, 1, 0, 0))
            dst = _table(n, (0, 1, 1, 0, 0, 0, 0))
            sign = jnp.asarray(_table(n, (0, 0, 1, 1, -1, 1, -1)), f32)

            def raw(a, k, j):
                rows = pl.ds(_mult((4 * j + 2 * (a >> 1) + (k >> 1)) * 64, 64), 64)
                return _unpack(w4b[a & 1, rows, pl.ds((k & 1) * C4, C4)]).astype(f32)

            def w(k):
                return jnp.concatenate(
                    [raw(i0, k, j) + sg * raw(i1, k, j) for j in range(NJ)], axis=0)

            def product(q):
                lhs = _comb(LHS[q], lambda k: jnp.concatenate(
                    [hid[p, k, j] for j in range(NJ)], axis=1))
                return _dot(lhs.astype(bf16), _comb(RHS[q], w).astype(bf16))

            def rows(k, i):
                return pl.ds(_mult(i * RB + (2 * (t >> 1) + (k >> 1)) * QB, QB), QB)

            def gather(ref, c, k):
                return jnp.concatenate([ref[c, rows(k, i), :] for i in range(S // RB)], axis=0)

            opens = _table(n, (1, 0, 1, 1, 0, 1, 0)) > 0

            @functools.cache
            def base(k):
                return (gather(hs_[k & 1], t & 1, k)
                        + jnp.where(opens, gather(xn[k & 1], t & 1, k), 0.0)
                        + jnp.where(n > 1, sign * prev[k][src], 0.0))

            if not last:
                for k in range(4):
                    base(k)

            def emit(k, v):
                v = 0.5 * v
                if not last:
                    prev[k][dst] = v
                v = v + base(k)
                for i in range(S // RB):
                    vi = v[i * QB:(i + 1) * QB]
                    if not last:
                        hs_[k & 1][t & 1, rows(k, i), :] = vi
                    stage[t, i, pl.ds((k >> 1) * QB, QB), pl.ds((k & 1) * C4, C4)] = (
                        vi.astype(bf16))

                if last:
                    for done in {1: (2, 1), 0: (3, 0)}.get(k, ()):
                        out_copy(t, done).start()

            _assemble_lazy(product, emit)
            return t

        @pl.loop(0, 6)
        def _(n):
            pl.when((n == 2) | (n > 3))(out_copy(down(n)).start)

        down(6, last=True)
        for t in range(4):
            out_copy(t).wait()

    pl.run_scoped(
        mlp,
        pltpu.VMEM((7, 4, NJ, S // 4, 128), f32),
        pltpu.VMEM((4, S // RB, RB // 2, D // 2), bf16),
        *[pltpu.VMEM((2, S // 4, C4), f32)] * 4)


@jax.jit
def pallas_sequential_preLN__memory_aug_recurrent_mem_tr__mixer_s_mlp__prompt_kernel(
    A_x: jax.Array,
    A_mem0: jax.Array,
    A_Wq: jax.Array,
    A_Wk: jax.Array,
    A_Wv: jax.Array,
    A_Wo: jax.Array,
    A_seg_len: jax.Array,
    B_x: jax.Array,
    B_w1: jax.Array,
    B_w2: jax.Array,
    B_w3: jax.Array,
    B_w4: jax.Array,
):
    del A_seg_len, B_x
    hbm = pl.BlockSpec(memory_space=pl.ANY)
    vmem = pl.BlockSpec(memory_space=pltpu.VMEM)
    scratch = [
        pltpu.VMEM((2, S, C4), f32),
        pltpu.VMEM((2, S, C4), f32),
        pltpu.VMEM((2, S, C4), f32),
        pltpu.VMEM((2, S, C4), f32),
        pltpu.VMEM((4 * NJ * D // 2, 128), u32),
        pltpu.VMEM((2, F // 2, 512), u32),
        pltpu.SemaphoreType.DMA((NSEM,)),
    ] + [pltpu.VMEM((H // 8, RING, DH), f32)] * 16
    out = pl.pallas_call(
        _kernel,
        out_shape=jax.ShapeDtypeStruct((S // RB, 2, RB // 2, D), A_x.dtype),
        in_specs=[hbm, vmem] + [hbm] * 8,
        out_specs=hbm,
        scratch_shapes=scratch,
        compiler_params=pltpu.CompilerParams(vmem_limit_bytes=128 * 1024 * 1024),
    )(A_x.reshape(S, D), A_mem0.reshape(MEM, D),
      A_Wq.reshape(D // 2, 2 * H, DH), A_Wk.reshape(D // 2, 2 * H, DH),
      A_Wv.reshape(D // 2, 2 * H, DH),
      A_Wo.reshape(H * DH, D), B_w1, B_w2, B_w3, B_w4)
    return out.reshape(A_x.shape)
```

```python
import functools

import jax
import jax.numpy as jnp
from jax import lax
import jax.experimental.pallas as pl
import jax.experimental.pallas.tpu as pltpu

S = 2048
D = 1024
H = 32
DH = 128
MEM = 8
SEG = 32
F = 3584
NSEG = S // SEG
L = MEM + SEG
TOK = 24
P0 = S - TOK * NSEG
RING = 576
XN = 48
C4 = D // 4
HALO = 8
RB = 256
QB = RB // 4
NJ = F // 512
EPS = 1e-5
NEG = -1000000000.0

LAG_QK, LAG_PV, LAG_WO = 2, 4, 6
SPLIT = 5
UNROLL = 2

bf16 = jnp.bfloat16
f32 = jnp.float32
u32 = jnp.uint32

SEM_X0, SEM_X, SEM_WO, SEM_W1, SEM_W2, SEM_W3, SEM_W4, SEM_OUT, SEM_W = (
    0, 1, 5, 9, 13, 14, 15, 16, 20)
NSEM = SEM_W + 12


def _mult(i, n):
    return i if isinstance(i, int) else pl.multiple_of(i, n)


def _ln(x):
    m = jnp.mean(x, axis=-1, keepdims=True)
    d = x - m
    v = jnp.mean(d * d, axis=-1, keepdims=True)
    return d * lax.rsqrt(v + EPS)


def _gelu2(x):
    k = 0.7978845608028654
    return x + x * jnp.tanh(x * (k + (k * 0.044715) * (x * x)))


def _pack(x):
    return pltpu.bitcast(x.astype(bf16), u32)


def _unpack(x):
    return pltpu.bitcast(x, bf16)


def _dot(a, b):
    return jnp.dot(a, b, preferred_element_type=f32)


LHS = ((0, 3, 1), (2, 3, 1), (0, 0, 0), (3, 3, 0), (0, 1, 1), (2, 0, -1), (1, 3, -1))
RHS = ((0, 3, 1), (0, 0, 0), (1, 3, -1), (2, 0, -1), (3, 3, 0), (0, 1, 1), (2, 3, 1))
ORDER = (0, 3, 1, 5, 2, 4, 6)


LAZY = (1, 3, 4, 2, 0, 5, 6)


def _comb(pat, block):
    i, j, sign = pat
    if sign == 0:
        return block(i)
    return block(i) + block(j) if sign > 0 else block(i) - block(j)


def _rc(i, k):
    return 2 * (i >> 1) + (k >> 1), 2 * (i & 1) + (k & 1)


def _assemble(product, emit=lambda k, v: None):
    m1 = product(0)
    m4 = product(3)
    c11 = m1 + m4
    m2 = product(1)
    c21 = m2 + m4
    c22 = m1 - m2
    c22 = c22 + product(5)
    emit(2, c21)
    m3 = product(2)
    c22 = c22 + m3
    m5 = product(4)
    emit(3, c22)
    c12 = m3 + m5
    c11 = c11 - m5
    c11 = c11 + product(6)
    emit(1, c12)
    emit(0, c11)
    return c11, c12, c21, c22


def _assemble_lazy(product, emit=lambda k, v: None):
    m2 = product(1)
    m4 = product(3)
    c21 = m2 + m4
    m5 = product(4)
    emit(2, c21)
    c11 = m4 - m5
    m3 = product(2)
    c12 = m3 + m5
    c22 = m3 - m2
    m1 = product(0)
    emit(1, c12)
    c11 = c11 + m1
    c22 = c22 + m1
    c22 = c22 + product(5)
    c11 = c11 + product(6)
    emit(3, c22)
    emit(0, c11)
    return c11, c12, c21, c22


def _operands(pats, block):
    for p in range(7):
        outer = [_comb(pats[p], lambda a: block(*_rc(a, k))) for k in range(4)]
        for q in range(7):
            yield 7 * p + q, _comb(pats[q], lambda k: outer[k])


def _two_level(product, emit, inner=_assemble_lazy):
    def outer(p):
        return jnp.concatenate(inner(lambda q: product(p, q)), axis=0)

    def done(a, v):
        n = v.shape[0] // 4
        for k in (2, 1, 3, 0) if inner is _assemble_lazy else (2, 3, 1, 0):
            emit(*_rc(a, k), v[k * n:(k + 1) * n])

    _assemble_lazy(outer, done)


def _operand(pats, block):
    @functools.cache
    def outer(p, k):
        return _comb(pats[p], lambda a: block(*_rc(a, k)))

    return lambda p, q: _comb(pats[q], lambda k: outer(p, k)).astype(bf16)


def _table(i, vals):
    if isinstance(i, int):
        return vals[i]
    r = jnp.int32(vals[-1])
    for k in range(len(vals) - 2, -1, -1):
        r = jnp.where(i == k, vals[k], r)
    return r


def _attention_and_mixer(x_hbm, mem0_ref, wq_hbm, wk_hbm, wv_hbm, wo_hbm, w1_hbm, w2_hbm,
                         w3_hbm, w4_hbm, hs_, xn, kv_rings, w3b, w4b, sems,
                         wo_b, xg, w1b, w2b, *q_rings):
    w_hbm = (wq_hbm, wk_hbm, wv_hbm)
    q_r = [q_rings[h % 8].at[h // 8] for h in range(H)]

    def h_load(rows):
        return jnp.concatenate([hs_[c & 1][c >> 1, rows, :] for c in range(4)], axis=1)

    def h_store(rows, v):
        for c in range(4):
            hs_[c & 1][c >> 1, rows, :] = v[:, c * C4:(c + 1) * C4]

    def wo_copy(i):
        rows = pl.ds(_mult(i * 512, 512), 512)
        return pltpu.make_async_copy(wo_hbm.bitcast(u32).at[rows], wo_b.at[rows],
                                     sems.at[SEM_WO + i])

    mlp_copies = [
        pltpu.make_async_copy(w3_hbm.bitcast(u32).at[:, pl.ds(j * 128, 128)],
                              w3b.at[pl.ds(j * D // 2, D // 2)],
                              sems.at[SEM_W3]) for j in range(4 * NJ)] + [
        pltpu.make_async_copy(w1_hbm.bitcast(u32), w1b, sems.at[SEM_W1]),
        pltpu.make_async_copy(w2_hbm.bitcast(u32), w2b, sems.at[SEM_W2])]

    def x_copies(r0, n, sem):
        rows = pl.ds(_mult(r0 // 2, 64), n // 2)
        return [pltpu.make_async_copy(x_hbm.bitcast(u32).at[rows, pl.ds(e * 512, 512)],
                                      w4b.at[e, rows], sems.at[sem]) for e in range(2)]

    def norm_x(r0, n):
        rows = pl.ds(_mult(r0 // 2, 8), n // 2)
        xv = jnp.concatenate([_unpack(w4b[e, rows, :]) for e in range(2)], axis=1).astype(f32)
        h_store(pl.ds(_mult(r0, 8), n), xv)
        return _ln(xv)

    def norm_tokens(r0, n):
        xg[pl.ds(_mult(r0, 8), n), :] = norm_x(r0, n)

    def prologue(w_s, rings, lhs0):
        pitch = 4 * D + 64
        stg = [w3b.at[pl.ds(m * pitch, 4 * D)] for m in range(3)]

        def start_chunk(g, m):
            src = w_hbm[m].bitcast(u32)
            dst = w3b.reshape(w3b.shape[0] // 8, 8, DH)
            for par in range(2):
                pltpu.make_async_copy(
                    src.at[:, pl.ds(_mult(16 * par + 4 * g, 4), 4), :],
                    dst.at[pl.ds(m * pitch // 8, D // 2), pl.ds(4 * par, 4), :],
                    sems.at[SEM_W + 3 * g + m]).start()

        def wait_chunk(g, m):
            pltpu.make_async_copy(stg[m], stg[m], sems.at[SEM_W + 3 * g + m]).wait()

        def x_part(g):
            return x_copies(P0 + g * ((S - P0) // 4), (S - P0) // 4, SEM_X + g)

        x0 = x_copies(0, P0, SEM_X0)
        for c in x0:
            c.start()
        start_chunk(0, 0)
        for c in x0:
            c.wait()
        start_chunk(0, 1)

        @pl.loop(0, P0 // 4 // 32)
        def _(i):
            y = [norm_x(r * (P0 // 4) + 32 * i, 32) for r in range(4)]
            for e in range(2):
                for n, v in _operands(LHS, lambda r, c: y[r][:, c * C4 + e * 128:][:, :128]):
                    lhs0[n, pl.ds(pl.multiple_of(16 * i, 16), 16), pl.ds(e * 128, 128)] = _pack(v)

        start_chunk(0, 2)
        wait_chunk(0, 0)
        for c in x_part(3):
            c.start()

        def stage(g, m):
            count = [0]
            for e in range(2):
                seen = []

                def block(r, c):
                    at = (8 * g + 4 * e + c, pl.ds(r * C4 // 2, C4 // 2), slice(None))
                    if (r, c) in seen:
                        return _unpack(w_s[m][at]).astype(f32)
                    seen.append((r, c))
                    w = w3b[pl.ds(m * pitch + 4 * C4 * r + 2 * e + (c >> 1), C4, stride=4), :]
                    w = pltpu.bitcast(w & jnp.uint32(0xFFFF0000) if c & 1 else w << 16, f32)
                    w_s[m][at] = _pack(w)
                    return w

                b = _operand(RHS, block)

                def product(p, q):
                    res = _dot(_unpack(lhs0[7 * p + q]), b(p, q))
                    k = count[0]
                    count[0] += 1
                    if k == 73 and m < 2:
                        wait_chunk(g, m + 1)
                        if m == 1:
                            pl.when(g < 3)(functools.partial(start_chunk, g + 1, 0))
                    return res

                def emit(r, c, v):
                    rings[m * 8 + 4 * e + c][g, pl.ds(r * (P0 // 4), P0 // 4), :] = v

                _two_level(product, emit)


        @pl.loop(0, 4)
        def _(g):
            for m in range(3):
                stage(g, m)

            @pl.when(g < 3)
            def _():
                start_chunk(g + 1, 1)
                start_chunk(g + 1, 2)
                wo_copy(g).start()
                for c in x_part(g):
                    c.start()
                wait_chunk(g + 1, 0)

            pl.when(g == 2)(wo_copy(3).start)

        for g in range(4):
            for c in x_part(g):
                c.wait()
        norm_tokens(P0, XN)

    def wrap(r):
        return jnp.where(r >= RING, r - RING, r)

    def mixer_norm(r0, n):
        h = h_load(pl.ds(r0, n))
        d = h - jnp.mean(h, axis=-1, keepdims=True)
        var = jnp.mean(d * d, axis=-1, keepdims=True)
        inv = lax.rsqrt(var + EPS)
        v = d * inv
        for c in range(4):
            xn[c & 1][c >> 1, pl.ds(r0, n), :] = v[:, c * C4:(c + 1) * C4]
        xg[pl.ds(r0, n), :] = v * lax.rsqrt(var * inv * inv + EPS)

    def load_tok(s):
        return xg[pl.ds(pl.multiple_of(P0 + TOK * s, 8), TOK), :]

    def step(w_s, ring, s, carry, tok):
        mem, rp, ra, rw = carry
        def head_pos(axis):
            i = lax.broadcasted_iota(jnp.int32, (2 * L, 2 * L), axis)
            second = ((i >= MEM) & (i < 2 * MEM)) | (i >= 2 * MEM + SEG)
            return second, i
        (rh, ri), (ch, ci) = head_pos(0), head_pos(1)
        same = rh == ch
        mask = same & ((ri < 2 * MEM) | (ri >= ci))
        masked = jnp.where(same, NEG, -jnp.inf)

        lhs = jnp.concatenate([mem, tok], axis=0).astype(bf16)
        rps = [pl.multiple_of(wrap(rp + 8 * i), 8) for i in range(3)]
        ra_ = pl.multiple_of(ra, SEG)
        rw_ = pl.multiple_of(rw, 8)

        mem_qkv = {}
        scores = {}
        o_mem = {}
        total = [None]
        late = []

        half = D // 2
        early = {}
        for i in range(SPLIT):
            early[i // 3, i % 3] = _dot(lhs[:, :half], _unpack(w_s[i % 3][i // 3, :half // 2]))

        def qkv(h):
            res = []
            for m in range(3):
                if (h, m) in early:
                    r = _dot(lhs[:, half:], _unpack(w_s[m][h, half // 2:])) + early[h, m]
                else:
                    r = _dot(lhs, _unpack(w_s[m][h]))
                for i in range(3):
                    ring[m][h][pl.ds(rps[i], 8), :] = r[8 + 8 * i:16 + 8 * i]
                res.append(r[:MEM])
            mem_qkv[h] = res

        def both(m, h):
            return jnp.concatenate(
                [mem_qkv[h][m], mem_qkv[h + 1][m], ring[m][h][pl.ds(ra_, SEG), :],
                 ring[m][h + 1][pl.ds(ra_, SEG), :]], axis=0).astype(bf16)

        def qk(h):
            scores[h] = lax.dot_general(both(0, h), both(1, h), (((1,), (1,)), ((), ())),
                                        preferred_element_type=f32)

        def pv(h):
            va = both(2, h)
            sc = jnp.where(mask, scores.pop(h) * (DH ** -0.5), masked)
            mx = jnp.max(sc, axis=1, keepdims=True)
            e = jnp.exp(sc - mx)
            den = jnp.sum(e, axis=1, keepdims=True)
            inv = pl.reciprocal(den, approx=True)
            inv = inv * (2.0 - den * inv)
            o = _dot(e.astype(bf16), va) * inv
            for i in range(2):
                q_r[h + i][pl.ds(ra_, SEG), :] = o[2 * MEM + i * SEG:2 * MEM + (i + 1) * SEG]
                o_mem[h + i] = o[i * MEM:(i + 1) * MEM]

        def wo(h):
            lo = jnp.concatenate([o_mem.pop(h), q_r[h][pl.ds(rw_, TOK), :]],
                                 axis=0).astype(bf16)
            rows = pl.ds(h * DH // 2, DH // 2)
            if h >= H - SPLIT:
                if not late:
                    total[:] = [total[0][:, :half], total[0][:, half:]]
                late.append((lo, rows))
                total[0] = total[0] + _dot(lo, _unpack(wo_b[rows, :half]))
                return
            r = _dot(lo, _unpack(wo_b[rows, :]))
            total[0] = r if total[0] is None else total[0] + r

        npair = H // 2
        for t in range(npair + LAG_WO):
            if 0 <= t - LAG_QK < npair:
                qk(2 * (t - LAG_QK))
            if 0 <= t - LAG_PV < npair:
                pv(2 * (t - LAG_PV))
            if t < npair:
                qkv(2 * t)
                qkv(2 * t + 1)
            if 0 <= t - LAG_WO < npair:
                wo(2 * (t - LAG_WO))
                wo(2 * (t - LAG_WO) + 1)
        for lo, rows in late:
            total[1] = total[1] + _dot(lo, _unpack(wo_b[rows, half:]))
        a = jnp.concatenate(total, axis=1)
        rows = pl.ds(pl.multiple_of(TOK * s, 8), TOK)
        h_store(rows, h_load(rows) + a[MEM:])
        return a[:MEM], wrap(rp + TOK), wrap(ra + SEG), wrap(rw + TOK)

    def block_a(lhs0, wq_s, wk_s, wv_s):
        w_s = (wq_s, wk_s, wv_s)
        rings = q_rings + kv_rings
        ring = [[rings[m * 8 + h % 8].at[h // 8] for h in range(H)] for m in range(3)]
        prologue(w_s, rings, lhs0)
        for i in range(4):
            wo_copy(i).wait()
        for c in mlp_copies:
            c.start()

        def steps(i, carry):
            s0 = i * UNROLL
            toks = [load_tok(s0 + k) for k in range(UNROLL)]
            behind = jnp.maximum(s0 - UNROLL, 0) * TOK
            ahead = jnp.minimum(P0 + (i + 1) * XN, S - XN)
            for k in range(UNROLL):
                mixer_norm(pl.multiple_of(behind + TOK * k, 8), TOK)
            for k in range(UNROLL):
                if k == UNROLL - 1:
                    norm_tokens(ahead, XN)
                carry = step(w_s, ring, s0 + k, carry, toks[k])
            return carry

        carry = (mem0_ref[...].astype(f32), jnp.int32(P0), jnp.int32(0), jnp.int32(0))
        lax.fori_loop(0, NSEG // UNROLL, steps, carry)
        for c in mlp_copies:
            c.wait()

    pl.run_scoped(block_a, pltpu.VMEM((49, P0 // 8, C4), u32),
                  *[pltpu.VMEM((H, D // 2, DH), u32)] * 3)

    def mixer(gs):
        done = TOK * NSEG

        def wo_batch():
            n = (S - done) // 4

            def lhs(r, c):
                r0 = (done + r * n) % RING
                cut = min(n, RING - r0)
                return jnp.concatenate([jnp.concatenate(
                    [ref[c, pl.ds(r0, cut), :]] + ([ref[c, pl.ds(0, n - cut), :]] if cut < n else []),
                    axis=0) for ref in q_rings], axis=1)

            a = _operand(LHS, lhs)
            b = _operand(RHS, lambda r, c: _unpack(
                wo_b[pl.ds(r * 512, 512), pl.ds(c * C4, C4)]).astype(f32))

            def emit(r, c, v):
                hs_[c & 1][c >> 1, pl.ds(done + r * n, n), :] += v

            _two_level(lambda p, q: _dot(a(p, q), b(p, q)), emit)

        def mixer_dot(first, lhs, w, emit):
            a = _operand(LHS, lambda r, c: jnp.concatenate(
                [lhs(first(r, i), c) for i in range(S // RB)], axis=0))
            b = _operand(RHS, lambda r, c: _unpack(
                w[pl.ds(r * C4 // 2, C4 // 2), pl.ds(c * C4, C4)]).astype(f32))

            def split(r, c, v):
                for i in range(S // RB):
                    for e in range(2):
                        emit(first(r, i), 2 * c + e,
                             v[i * QB:(i + 1) * QB, e * 128:(e + 1) * 128])

            _two_level(lambda p, q: _dot(a(p, q), b(p, q)), split, _assemble)

        def mixer_in():
            def emit(r0, e, v):
                gs[e, pl.ds(HALO + r0, QB), :] = _gelu2(v)

            mixer_dot(lambda r, i: (3 - r) * S // 4 + i * QB,
                      lambda r0, c: xg[pl.ds(r0, QB), pl.ds(c * C4, C4)], w1b, emit)

        def mixer_out():
            def shifted(r0, c):
                rows = pl.ds(HALO + r0 + (-1, 1, -2, 2)[c], QB)
                return jnp.concatenate([gs[2 * c + e, rows, :] for e in range(2)], axis=1)

            def emit(r0, e, v):
                ref, at = xn[e >> 1 & 1], (e >> 2, pl.ds(r0, QB), pl.ds((e & 1) * 128, 128))
                x1[r0, e] = ref[at] + 0.5 * v
                ref[at] = x1[r0, e]

            x1 = {}
            mixer_dot(lambda r, i: i * RB + r * QB, shifted, w2b, emit)
            for i in range(S // RB):
                for u in range(0, QB, 8):
                    mixer_post(i, u, lambda r0, e: x1[r0, e][u:u + 8])

        def mixer_post(i, u, x1):
            y = {r: _ln(jnp.concatenate([x1(i * RB + r * QB, e) for e in range(8)], axis=1))
                 for r in (3, 2, 1, 0)}
            for k in range(4):
                blocks = [y[r][:, c * C4:(c + 1) * C4] for r, c in (_rc(a, k) for a in range(4))]
                for p in range(7):
                    v = _comb(LHS[p], lambda a: blocks[a])
                    for e in range(2):
                        kv_rings[2 * p + e][k, pl.ds(_mult(i * QB + u, 8), 8), :] = (
                            v[:, e * 128:(e + 1) * 128])

        for c in range(8):
            for r0 in (0, HALO + S):
                gs[c, pl.ds(r0, HALO), :] = jnp.zeros((HALO, 128), f32)
        mixer_norm(done - UNROLL * TOK, UNROLL * TOK)
        wo_batch()
        for r0 in range(done, S, 64):
            mixer_norm(r0, 64)
        mixer_in()
        mixer_out()

    pl.run_scoped(mixer, pltpu.VMEM((8, S + 2 * HALO, 128), f32))


def _kernel(*refs):
    inputs, out_hbm, (h0, h1, n0, n1, w3b, w4b, sems, *kv_rings) = refs[:10], refs[10], refs[11:]
    hs_, xn = (h0, h1), (n0, n1)
    pl.run_scoped(
        functools.partial(_attention_and_mixer, *inputs, hs_, xn, tuple(kv_rings), w3b, w4b, sems),
        pltpu.VMEM((H * DH // 2, D), u32),
        pltpu.VMEM((S, D), f32),
        pltpu.VMEM((D // 2, D), u32),
        pltpu.VMEM((D // 2, D), u32),
        *[pltpu.VMEM((H // 8, RING, DH), f32)] * 8)

    def mlp(hid, stage, *prev):
        w4_copies = [
            pltpu.make_async_copy(inputs[9].bitcast(u32).at[:, pl.ds(e * 512, 512)], w4b.at[e],
                                  sems.at[SEM_W4]) for e in range(2)]

        def up(j):
            def raw(a, k):
                r, c = _rc(a, k)
                rows = pl.ds(_mult((4 * j + c) * (D // 2) + r * 128, 128), 128)
                return _unpack(w3b[rows, :]).astype(f32)

            def y(p, k):
                return jnp.concatenate(
                    [kv_rings[2 * p + e][k, pl.ds(0, S // 4), :] for e in range(2)], axis=1)

            parts = {}
            for p in LAZY:
                w = [_comb(RHS[p], lambda a: raw(a, k)) for k in range(4)]
                parts[p] = _assemble_lazy(lambda q: _dot(
                    _comb(LHS[q], lambda k: y(p, k)).astype(bf16),
                    _comb(RHS[q], lambda k: w[k]).astype(bf16)))
            for k in (2, 3, 1, 0):
                for r0 in range(0, S // 4, 16):
                    g = [_gelu2(v) for v in _assemble_lazy(lambda p: parts[p][k][r0:r0 + 16])]
                    for p in range(7):
                        hid[p, k, j, pl.ds(r0, 16), :] = _comb(LHS[p], lambda a: g[a])

        @pl.loop(0, NJ)
        def _(j):
            @pl.when(j == 1)
            def _():
                for c in w4_copies:
                    c.start()

            up(j)

        def out_copy(t, k=None):
            r0, nr, c0, nc = (0, 2 * QB, 0, 2 * C4) if k is None else (
                (k >> 1) * QB, QB, (k & 1) * C4, C4)
            return pltpu.make_async_copy(
                stage.at[t, :, pl.ds(r0, nr), pl.ds(c0, nc)],
                out_hbm.at[:, t >> 1, pl.ds(r0, nr), pl.ds(_mult((t & 1) * 2 * C4 + c0, C4), nc)],
                sems.at[SEM_OUT + t])

        for c in w4_copies:
            c.wait()

        def down(n, last=False):
            p = _table(n, ORDER)
            i0, i1, sg = [_table(n, [RHS[o][e] for o in ORDER]) for e in range(3)]
            sg = jnp.asarray(sg, f32)
            t = _table(n, (0, 0, 2, 3, 3, 1, 0))
            src = _table(n, (0, 0, 1, 0, 1, 0, 0))
            dst = _table(n, (0, 1, 1, 0, 0, 0, 0))
            sign = jnp.asarray(_table(n, (0, 0, 1, 1, -1, 1, -1)), f32)

            def raw(a, k, j):
                rows = pl.ds(_mult((4 * j + 2 * (a >> 1) + (k >> 1)) * 64, 64), 64)
                return _unpack(w4b[a & 1, rows, pl.ds((k & 1) * C4, C4)]).astype(f32)

            def w(k):
                return jnp.concatenate(
                    [raw(i0, k, j) + sg * raw(i1, k, j) for j in range(NJ)], axis=0)

            def product(q):
                lhs = _comb(LHS[q], lambda k: jnp.concatenate(
                    [hid[p, k, j] for j in range(NJ)], axis=1))
                return _dot(lhs.astype(bf16), _comb(RHS[q], w).astype(bf16))

            def rows(k, i):
                return pl.ds(_mult(i * RB + (2 * (t >> 1) + (k >> 1)) * QB, QB), QB)

            def gather(ref, c, k):
                return jnp.concatenate([ref[c, rows(k, i), :] for i in range(S // RB)], axis=0)

            opens = _table(n, (1, 0, 1, 1, 0, 1, 0)) > 0

            @functools.cache
            def base(k):
                return (gather(hs_[k & 1], t & 1, k)
                        + jnp.where(opens, gather(xn[k & 1], t & 1, k), 0.0)
                        + jnp.where(n > 1, sign * prev[k][src], 0.0))

            if not last:
                for k in range(4):
                    base(k)

            def emit(k, v):
                v = 0.5 * v
                if not last:
                    prev[k][dst] = v
                v = v + base(k)
                for i in range(S // RB):
                    vi = v[i * QB:(i + 1) * QB]
                    if not last:
                        hs_[k & 1][t & 1, rows(k, i), :] = vi
                    stage[t, i, pl.ds((k >> 1) * QB, QB), pl.ds((k & 1) * C4, C4)] = (
                        vi.astype(bf16))

                if last:
                    for done in {1: (2, 1), 0: (3, 0)}.get(k, ()):
                        out_copy(t, done).start()

            _assemble_lazy(product, emit)
            return t

        @pl.loop(0, 6)
        def _(n):
            pl.when((n == 2) | (n > 3))(out_copy(down(n)).start)

        down(6, last=True)
        for t in range(4):
            out_copy(t).wait()

    pl.run_scoped(
        mlp,
        pltpu.VMEM((7, 4, NJ, S // 4, 128), f32),
        pltpu.VMEM((4, S // RB, RB // 2, D // 2), bf16),
        *[pltpu.VMEM((2, S // 4, C4), f32)] * 4)


@jax.jit
def pallas_sequential_preLN__memory_aug_recurrent_mem_tr__mixer_s_mlp__prompt_kernel(
    A_x: jax.Array,
    A_mem0: jax.Array,
    A_Wq: jax.Array,
    A_Wk: jax.Array,
    A_Wv: jax.Array,
    A_Wo: jax.Array,
    A_seg_len: jax.Array,
    B_x: jax.Array,
    B_w1: jax.Array,
    B_w2: jax.Array,
    B_w3: jax.Array,
    B_w4: jax.Array,
):
    del A_seg_len, B_x
    hbm = pl.BlockSpec(memory_space=pl.ANY)
    vmem = pl.BlockSpec(memory_space=pltpu.VMEM)
    scratch = [
        pltpu.VMEM((2, S, C4), f32),
        pltpu.VMEM((2, S, C4), f32),
        pltpu.VMEM((2, S, C4), f32),
        pltpu.VMEM((2, S, C4), f32),
        pltpu.VMEM((4 * NJ * D // 2, 128), u32),
        pltpu.VMEM((2, F // 2, 512), u32),
        pltpu.SemaphoreType.DMA((NSEM,)),
    ] + [pltpu.VMEM((H // 8, RING, DH), f32)] * 16
    out = pl.pallas_call(
        _kernel,
        out_shape=jax.ShapeDtypeStruct((S // RB, 2, RB // 2, D), A_x.dtype),
        in_specs=[hbm, vmem] + [hbm] * 8,
        out_specs=hbm,
        scratch_shapes=scratch,
        compiler_params=pltpu.CompilerParams(vmem_limit_bytes=128 * 1024 * 1024),
    )(A_x.reshape(S, D), A_mem0.reshape(MEM, D),
      A_Wq.reshape(D // 2, 2 * H, DH), A_Wk.reshape(D // 2, 2 * H, DH),
      A_Wv.reshape(D // 2, 2 * H, DH),
      A_Wo.reshape(H * DH, D), B_w1, B_w2, B_w3, B_w4)
    return out.reshape(A_x.shape)
```
